```python
import jax
import jax.numpy as jnp

def _softmax(x, axis=-1):
    return jax.nn.softmax(x, axis=axis)

def _gelu(x):
    return jax.nn.gelu(x, approximate=True)

def _silu(x):
    return jax.nn.silu(x)

def _sigmoid(x):
    return jax.nn.sigmoid(x)

def _layernorm(x, axis=-1, eps=1e-05):
    m = jnp.mean(x, axis=axis, keepdims=True)
    v = jnp.var(x, axis=axis, keepdims=True)
    return (x - m) / jnp.sqrt(v + eps)

def _scatter_add(tgt, idx, src, axis=0):
    return tgt.at[idx].add(src)

def _segment_sum(src, seg, n):
    return jax.ops.segment_sum(src, seg, n)

class _Rng:

    def __init__(self, key):
        self._k = key

    def _next(self):
        self._k, sub = jax.random.split(self._k)
        return sub

    def normal(self, shape):
        return jax.random.normal(self._next(), shape, dtype=jnp.bfloat16)

    def randint(self, lo, hi, shape):
        return jax.random.randint(self._next(), shape, lo, hi, dtype=jnp.int32)

    def uniform(self, shape, lo=0.0, hi=1.0):
        return jax.random.uniform(self._next(), shape, jnp.bfloat16, lo, hi)

    def permutation(self, n):
        return jax.random.permutation(self._next(), n)
kernel_name = 'parallel_sum__memory_aug_infini_attn__moe_arch_mod__prompt'

def setup_inputs():
    _rng = _Rng(jax.random.key(int.from_bytes(__import__("os").urandom(4), "little")))
    _w = lambda a: (lambda t: t.astype(jnp.bfloat16) if jnp.issubdtype(t.dtype, jnp.floating) else t)(jnp.asarray(a))

    def _A_setup():
        B, S, D, H = (1, 2048, 576, 32)
        N = 4
        L = max(1, S // N)
        sc = D ** (-0.5)
        return {'x': _w((lambda *s: _rng.normal(s) * 0.05)(B, N * L, D)), 'wq': _w((lambda *s: _rng.normal(s) * 0.05)(D, D) * sc), 'wk': _w((lambda *s: _rng.normal(s) * 0.05)(D, D) * sc), 'wv': _w((lambda *s: _rng.normal(s) * 0.05)(D, D) * sc), 'wo': _w((lambda *s: _rng.normal(s) * 0.05)(D, D) * sc), 'beta': _w((lambda *s: _rng.normal(s) * 0.05)(H))}
    _A_in = _A_setup()

    def _B_setup():
        B, S, D, F, C = (1, 2048, 576, 4608, 2)
        return {'x': _w((lambda *s: _rng.normal(s) * 0.05)(B, S, D)), 'w_r': _w((lambda *s: _rng.normal(s) * 0.05)(D)), 'w_gate': _w((lambda *s: _rng.normal(s) * 0.05)(D, F)), 'w_up': _w((lambda *s: _rng.normal(s) * 0.05)(D, F)), 'w_down': _w((lambda *s: _rng.normal(s) * 0.05)(F, D))}
    _B_in = _B_setup()
    return {'A_x': _A_in['x'], 'A_wq': _A_in['wq'], 'A_wk': _A_in['wk'], 'A_wv': _A_in['wv'], 'A_wo': _A_in['wo'], 'A_beta': _A_in['beta'], 'B_x': _B_in['x'], 'B_w_r': _B_in['w_r'], 'B_w_gate': _B_in['w_gate'], 'B_w_up': _B_in['w_up'], 'B_w_down': _B_in['w_down']}

def reference(A_x, A_wq, A_wk, A_wv, A_wo, A_beta, B_x, B_w_r, B_w_gate, B_w_up, B_w_down):

    def _A_ref(x, wq, wk, wv, wo, beta):
        B, S, D = x.shape
        H = 32
        Dh = D // H
        N = 4
        L = S // N
        q = (lambda x, *d: x.transpose(*d))((x @ wq).reshape(B, S, H, Dh), 0, 2, 1, 3).reshape(B, H, N, L, Dh)
        k = (lambda x, *d: x.transpose(*d))((x @ wk).reshape(B, S, H, Dh), 0, 2, 1, 3).reshape(B, H, N, L, Dh)
        v = (lambda x, *d: x.transpose(*d))((x @ wv).reshape(B, S, H, Dh), 0, 2, 1, 3).reshape(B, H, N, L, Dh)
        phi = lambda t: jnp.where(t > 0, t + 1.0, jnp.exp(t))
        scale = Dh ** (-0.5)
        ar = jnp.arange(L)
        mask = (lambda x, dt: x.astype(dt))(ar[:, None] < ar[None, :], x.dtype) * -1000000000.0
        g = _sigmoid(beta).reshape(1, H, 1, 1)
        M = jnp.einsum('bhd,bhe->bhde', q[:, :, 0, 0, :] * 0.0, q[:, :, 0, 0, :] * 0.0)
        z = q[:, :, 0, 0, :] * 0.0
        outs = []
        for s in range(N):
            qs, ks, vs = (q[:, :, s].copy(), k[:, :, s].copy(), v[:, :, s].copy())
            logits = jnp.einsum('bhqd,bhkd->bhqk', qs, ks) * scale + mask
            p = _softmax(logits, axis=-1)
            a_dot = jnp.einsum('bhqk,bhkd->bhqd', p, vs)
            pq = phi(qs)
            num = jnp.einsum('bhld,bhde->bhle', pq, M)
            den = jnp.einsum('bhld,bhd->bhl', pq, z)[..., None] + 1e-06
            a_mem = num / den
            o = g * a_mem + (1.0 - g) * a_dot
            outs.append(o)
            pk = phi(ks)
            M = M + jnp.einsum('bhld,bhle->bhde', pk, vs)
            z = z + jnp.einsum('bhld->bhd', pk)
        o = (lambda x, *d: x.transpose(*d))(jnp.stack(outs, 2).reshape(B, H, S, Dh), 0, 2, 1, 3).reshape(B, S, D)
        return o @ wo

    def _B_ref(x, w_r, w_gate, w_up, w_down):
        B, S, D = x.shape
        C = 2
        r = x @ w_r
        idx = jnp.argsort(-r, axis=-1)[:, :C]
        idx_e = jnp.repeat(idx.reshape(B, C, 1), D, axis=2)
        x_sel = jnp.take_along_axis(x, idx_e, axis=1)
        g = _silu(x_sel @ w_gate)
        u = x_sel @ w_up
        y = g * u @ w_down
        r_sel = _sigmoid(jnp.take_along_axis(r, idx, axis=1))
        y = y * r_sel.reshape(B, C, 1)
        b_off = (jnp.arange(B) * S).reshape(B, 1)
        flat_idx = (idx + b_off).reshape(B * C)
        zero = (x * 0.0).reshape(B * S, D)
        upd = _scatter_add(zero, flat_idx, y.reshape(B * C, D), axis=0)
        return x + upd.reshape(B, S, D)
    x = A_x
    xn = _layernorm(x, axis=-1)
    return x + _A_ref(xn, A_wq, A_wk, A_wv, A_wo, A_beta) + _B_ref(xn, B_w_r, B_w_gate, B_w_up, B_w_down)
```

```python
import math

import jax
import jax.numpy as jnp
import numpy as np
from jax import lax
import jax.experimental.pallas as pl
import jax.experimental.pallas.tpu as pltpu

S, D, H, DH, NSEG, L, F = 2048, 576, 32, 18, 4, 512, 4608
DP = D // 2
NW, WSTR = 5, 112
WIN_HEADS = ((0, 7), (7, 13), (13, 19), (19, 25), (25, 32))
NFC = 4
FC = F // NFC
LOG2E = math.log2(math.e)
QSCALE = DH ** -0.5 * LOG2E
NEG = -1e9 * LOG2E

f32, bf16, i32 = jnp.float32, jnp.bfloat16, jnp.int32


def _b(x):
    return pltpu.bitcast(x, bf16)


def _w(x):
    return pltpu.bitcast(x, i32)


def _rnd(x):
    return x.astype(bf16).astype(f32)


def _phi(t):
    return jnp.where(t > 0, t + 1.0, jnp.exp(t))


def _dot(a, b):
    return jnp.dot(a, b, preferred_element_type=f32)


def _dot_nt(a, b):
    return lax.dot_general(a, b, (((1,), (1,)), ((), ())), preferred_element_type=f32)


def _iota(shape, dim):
    return lax.broadcasted_iota(i32, shape, dim)


def _kernel(x_hbm, wq_hbm, wk_hbm, wv_hbm, wo_hbm, beta_ref, wr_ref, wg_hbm, wu_hbm, wd_hbm,
            out_hbm,
            xs, xn, wraw, wt, wot, qs, vt, kw, amem, mz, wg, wu, wd, obuf, rs, ot, adot, tri,
            gate, rden, sem_x, sem_w, sem_f, sem_o):
    x32 = x_hbm.bitcast(i32)
    out32 = out_hbm.bitcast(i32)

    def x_copy(s):
        return pltpu.make_async_copy(x32.at[:, pl.ds(s * L, L)], xs.at[s], sem_x.at[s])

    def w_copy(j):
        src = (wq_hbm, wk_hbm, wv_hbm, wo_hbm)[j]
        return pltpu.make_async_copy(src.bitcast(i32), wraw.at[j], sem_w.at[j])

    def f_copy(j, c):
        src, dst = ((wg_hbm, wg), (wu_hbm, wu), (wd_hbm, wd))[j]
        return pltpu.make_async_copy(src.bitcast(i32).at[:, pl.ds(c * FC, FC)], dst.at[c],
                                     sem_f.at[j * NFC + c])

    def o_copy(s):
        return pltpu.make_async_copy(obuf.at[s], out32.at[:, pl.ds(pl.multiple_of(s * L, L), L)],
                                     sem_o.at[s])

    x_copy(0).start()
    for j in range(3):
        w_copy(j).start()
    for s in range(1, NSEG):
        x_copy(s).start()
    w_copy(3).start()
    for c in range(NFC):
        for j in range(3):
            f_copy(j, c).start()

    tri[...] = jnp.where(_iota((128, 128), 0) > _iota((128, 128), 1), NEG, 0.0).astype(f32)
    beta = beta_ref[...].astype(f32).reshape(1, H)
    g_row = _rnd(jax.nn.sigmoid(beta))
    eye = _iota((H, H), 0) == _iota((H, H), 1)
    g_col = jnp.sum(jnp.where(eye, jnp.broadcast_to(g_row, (H, H)), 0.0), axis=1, keepdims=True)
    gate[...] = jnp.broadcast_to(g_col, (H, 128))

    def layernorm(s):
        x = _b(xs[s]).astype(f32)
        mean = jnp.sum(x, axis=0, keepdims=True) * (1.0 / D)
        xc = x - mean
        var = jnp.sum(xc * xc, axis=0, keepdims=True) * (1.0 / D)
        sd = _rnd(jnp.sqrt(_rnd(_rnd(var) + float(np.asarray(1e-5, dtype=bf16)))))
        xn[s] = _w((_rnd(x - _rnd(mean)) * (1.0 / sd)).astype(bf16))

    x_copy(0).wait()
    layernorm(0)
    for j in range(3):
        w_copy(j).wait()
        wt[j * DP:(j + 1) * DP, :] = _w(_b(wraw[j]).T)
    wr = wr_ref[...].astype(f32).reshape(1, D)
    wt[3 * DP:3 * DP + 8, :] = _w(jnp.broadcast_to(wr, (16, D)).astype(bf16))

    for s in range(NSEG):
        if s + 1 < NSEG:
            x_copy(s + 1).wait()
            layernorm(s + 1)
        xns = _b(xn[s])
        q = _dot(_b(wt[0:DP, :]), xns)
        qs[s] = _w((q * QSCALE).astype(bf16))
        if s > 0:
            pq = _phi(_rnd(q)).astype(bf16)
            nums = []
            for w, (h0, h1) in enumerate(WIN_HEADS):
                nd = _dot(mz[w].astype(bf16), pq[WSTR * w:WSTR * w + 128, :])
                nums.append(nd[0:128])
                rden[w] = nd[128:136]
            for w, (h0, h1) in enumerate(WIN_HEADS):
                gw = jnp.concatenate([gate[h0:h0 + 7, :], gate[0:1, :]], axis=0)
                rden[w] = jnp.tile(gw, (1, L // 128)) / (rden[w] + 1e-6)
            for rb in range(D // 8):
                ha, hb = (8 * rb) // DH, (8 * rb + 7) // DH

                def part(h):
                    w = min(max((h - 1) // 6, 0), NW - 1)
                    r0 = 8 * rb - WSTR * w
                    j = h - WIN_HEADS[w][0]
                    return nums[w][r0:r0 + 8], jnp.broadcast_to(rden[w, j:j + 1, :], (8, L))

                na, ra = part(ha)
                if ha == hb:
                    val = na * ra
                else:
                    nb, rb_ = part(hb)
                    val = jnp.where(_iota((8, L), 0) < DH * hb - 8 * rb, na * ra, nb * rb_)
                amem[s, 8 * rb:8 * rb + 8, :] = val
        else:
            amem[s] = jnp.zeros((D, L), f32)
        k = _dot(_b(wt[DP:2 * DP, :]), xns).astype(bf16)
        vr = _dot(_b(wt[2 * DP:3 * DP + 8, :]), xns)
        v = vr[0:D].astype(bf16)
        vt[s] = _w(v)
        rs[:, s * L:(s + 1) * L] = _rnd(vr[D:D + 8])
        for w, (h0, h1) in enumerate(WIN_HEADS):
            kwin = k[WSTR * w:WSTR * w + 128, :].T
            kw[s, w] = _w(kwin)
            if s + 1 < NSEG:
                pk = _phi(kwin.astype(f32)).astype(bf16)
                upd = _dot(v[WSTR * w:WSTR * w + 128, :], pk)
                zupd = jnp.sum(pk.astype(f32), axis=0, keepdims=True)
                same = None
                for h in range(h0, h1):
                    lo, hi = DH * h - WSTR * w, DH * (h + 1) - WSTR * w
                    r_, c_ = _iota((128, 128), 0), _iota((128, 128), 1)
                    m = (r_ >= lo) & (r_ < hi) & (c_ >= lo) & (c_ < hi)
                    same = m if same is None else (same | m)
                lo16 = DH * (_iota((16, 128), 0) + h0) - WSTR * w
                c16 = _iota((16, 128), 1)
                zmask = (c16 >= lo16) & (c16 < lo16 + DH)
                new = jnp.concatenate(
                    [jnp.where(same, upd, 0.0),
                     jnp.where(zmask, jnp.broadcast_to(zupd, (16, 128)), 0.0)], axis=0)
                mz[w] = new if s == 0 else mz[w] + new

    r = rs[...]
    tok = _iota((8, S), 1)
    m1 = jnp.max(r, axis=1, keepdims=True)
    i1 = jnp.min(jnp.where(r == m1, tok, S), axis=1, keepdims=True)
    r2 = jnp.where(tok == i1, -jnp.inf, r)
    m2 = jnp.max(r2, axis=1, keepdims=True)
    i2 = jnp.min(jnp.where((r2 == m2) & (tok != i1), tok, S), axis=1, keepdims=True)
    row = _iota((8, S), 0)
    sel8 = jnp.where(((row == 0) & (tok == i1)) | ((row == 1) & (tok == i2)), 1.0, 0.0)
    sel = jnp.concatenate([sel8, jnp.zeros((8, S), f32)], axis=0).astype(bf16)
    rsel8 = _rnd(jax.nn.sigmoid(jnp.where(_iota((8, 1), 0) == 0, m1, m2)))
    rsel = jnp.concatenate([rsel8, rsel8], axis=0)
    xsel = jnp.zeros((16, D), f32)
    for s in range(NSEG):
        xsel = xsel + _dot_nt(sel[:, s * L:(s + 1) * L], _b(xn[s]))
    xsel = xsel.astype(bf16)

    w_copy(3).wait()
    wot[:, 0:D] = _w(_b(wraw[3]).T)

    y = jnp.zeros((16, D), f32)
    for c in range(NFC):
        for j in range(3):
            f_copy(j, c).wait()
        g = _rnd(_dot(xsel, _b(wg[c])))
        u = _rnd(_dot(xsel, _b(wu[c])))
        hcat = (_rnd(g * jax.nn.sigmoid(g)) * u).astype(bf16)
        y = y + _dot_nt(hcat, _b(wd[c]))
    y = _rnd(_rnd(y) * rsel)
    ypad = jnp.concatenate([y, jnp.zeros((112, D), f32)], axis=0)
    wot[:, D:D + 64] = _w(ypad.T[:, 0:64].astype(bf16))

    ones_w = np.int32(0x3F803F80)

    def seg_body(s, carry):
        def head_body(h, carry):
            w = jnp.clip((h + 5) // 6 - 1, 0, NW - 1)
            prow = _iota((64, L), 0) + (WSTR // 2) * w
            qwin = qs[s, pl.ds(pl.multiple_of((WSTR // 2) * w, 8), 64), :]
            qm = _b(jnp.where((prow >= 9 * h) & (prow < 9 * h + 9), qwin, 0))
            a = (9 * h) // 8
            vrow = _iota((16, L), 0) + 8 * a
            vwin = vt[s, pl.ds(pl.multiple_of(8 * a, 8), 16), :]
            vm = _b(jnp.where((vrow >= 9 * h) & (vrow < 9 * h + 9), vwin, ones_w))
            orow = _iota((32, 128), 0) + 16 * a
            omask = (orow >= DH * h) & (orow < DH * h + DH)
            low = (DH * h - 16 * a) >= 8
            g1 = 1.0 - jnp.broadcast_to(gate[pl.ds(h, 1), :], (8, 128))
            for i in range(4):
                n = 128 * (i + 1)
                sc = _dot(_b(kw[s, w, 0:n // 2, :]), qm[:, 128 * i:128 * i + 128])
                diag = sc[n - 128:n] + tri[...]
                sc = diag if i == 0 else jnp.concatenate([sc[0:n - 128], diag], axis=0)
                m = jnp.max(sc, axis=0, keepdims=True)
                p = jnp.exp2(sc - m).astype(bf16)
                o = _dot(vm[:, 0:n], p)
                den = jnp.where(low, o[0:8], o[24:32])
                scale = g1 / den
                o = o * jnp.concatenate([scale] * 4, axis=0)
                pltpu.store(adot.at[pl.ds(pl.multiple_of(16 * a, 16), 32), 128 * i:128 * i + 128],
                            o, mask=omask)
            return carry

        lax.fori_loop(0, H, head_body, 0)
        ot[0:DP, :] = _w((amem[s] + adot[...]).astype(bf16))
        ot[DP:DP + 8, :] = _w(sel_ref[s])
        ot[DP + 8:, :] = jnp.zeros((24, L), i32)
        res = _dot(_b(wot[...]), _b(ot[...]))
        res = res + (_b(xs[s]).astype(f32) + _b(xn[s]).astype(f32))
        obuf[s] = _w(res.astype(bf16))
        o_copy(s).start()
        return carry

    def scoped(sel_ref_):
        nonlocal sel_ref
        sel_ref = sel_ref_
        for s in range(NSEG):
            sel_ref[s] = sel[:, s * L:(s + 1) * L]
        lax.fori_loop(0, NSEG, seg_body, 0)

    sel_ref = None
    pl.run_scoped(scoped, pltpu.VMEM((NSEG, 16, L), bf16))
    for s in range(NSEG):
        o_copy(s).wait()


@jax.jit
def pallas_parallel_sum__memory_aug_infini_attn__moe_arch_mod__prompt_kernel(
    A_x, A_wq, A_wk, A_wv, A_wo, A_beta, B_x, B_w_r, B_w_gate, B_w_up, B_w_down,
):
    hbm = pl.BlockSpec(memory_space=pl.ANY)
    vmem = pl.BlockSpec(memory_space=pltpu.VMEM)
    out = pl.pallas_call(
        _kernel,
        out_shape=jax.ShapeDtypeStruct((D, S), bf16),
        in_specs=[hbm, hbm, hbm, hbm, hbm, vmem, vmem, hbm, hbm, hbm],
        out_specs=hbm,
        scratch_shapes=[
            pltpu.VMEM((NSEG, DP, L), i32),
            pltpu.VMEM((NSEG, DP, L), i32),
            pltpu.VMEM((4, DP, D), i32),
            pltpu.VMEM((3 * DP + 8, D), i32),
            pltpu.VMEM((DP, 640), i32),
            pltpu.VMEM((NSEG, DP, L), i32),
            pltpu.VMEM((NSEG, DP, L), i32),
            pltpu.VMEM((NSEG, NW, L // 2, 128), i32),
            pltpu.VMEM((NSEG, D, L), f32),
            pltpu.VMEM((NW, 144, 128), f32),
            pltpu.VMEM((NFC, DP, FC), i32),
            pltpu.VMEM((NFC, DP, FC), i32),
            pltpu.VMEM((NFC, DP, FC), i32),
            pltpu.VMEM((NSEG, DP, L), i32),
            pltpu.VMEM((8, S), f32),
            pltpu.VMEM((320, L), i32),
            pltpu.VMEM((D, L), f32),
            pltpu.VMEM((128, 128), f32),
            pltpu.VMEM((H, 128), f32),
            pltpu.VMEM((NW, 8, L), f32),
            pltpu.SemaphoreType.DMA((NSEG,)),
            pltpu.SemaphoreType.DMA((4,)),
            pltpu.SemaphoreType.DMA((3 * NFC,)),
            pltpu.SemaphoreType.DMA((NSEG,)),
        ],
        compiler_params=pltpu.CompilerParams(vmem_limit_bytes=100 * 1024 * 1024),
        name="infini_mod",
    )(A_x[0].T, A_wq, A_wk, A_wv, A_wo, A_beta, B_w_r, B_w_gate, B_w_up, B_w_down.T)
    return out.T[None]
```

```python
import math

import jax
import jax.numpy as jnp
import numpy as np
from jax import lax
import jax.experimental.pallas as pl
import jax.experimental.pallas.tpu as pltpu

S, D, H, DH, NSEG, L, F = 2048, 576, 32, 18, 4, 512, 4608
DP = D // 2
GH, GR, GP = 8, 144, 72
NG = H // GH
NSTEP = NSEG * NG
FC = 512
NFC = F // FC
LOG2E = math.log2(math.e)
QSCALE = DH ** -0.5 * LOG2E
NEG = -1e9 * LOG2E
EPS_LN = float(np.asarray(1e-5, dtype=jnp.bfloat16))
ONES2 = np.int32(0x3F803F80)

f32, bf16, i32 = jnp.float32, jnp.bfloat16, jnp.int32


def _b(x):
    return pltpu.bitcast(x, bf16)


def _w(x):
    return pltpu.bitcast(x, i32)


def _rnd(x):
    return x.astype(bf16).astype(f32)


def _phi(t):
    return jnp.where(t > 0, t + 1.0, jnp.exp(t))


def _dot(a, b):
    return jnp.dot(a, b, preferred_element_type=f32)


def _dot_nt(a, b):
    return lax.dot_general(a, b, (((1,), (1,)), ((), ())), preferred_element_type=f32)


def _iota(shape, dim):
    return lax.broadcasted_iota(i32, shape, dim)


def _between(x, lo, hi):
    return (x >= lo) & (x < hi)


def _kernel(x_hbm, wq_hbm, wk_hbm, wv_hbm, wo_hbm, beta_ref, wr_ref, wg_hbm, wu_hbm, wd_hbm,
            out_hbm,
            xs, xn, wraw, wqt, wkt, wvt, wot, qs, pqs, kt, pkt, vt, kw, amem, adot, mz, mmask,
            wg, wu, wd, obuf, rs, tri, gate, gate1, rden, sel, xsel, rsel, hbuf, yacc,
            s_a, s_b, m_a, m_b,
            sem_x, sem_w, sem_f, sem_o):
    x32 = x_hbm.bitcast(i32)
    out32 = out_hbm.bitcast(i32)

    def x_copy(s):
        return pltpu.make_async_copy(x32.at[:, pl.ds(s * L, L)], xs.at[s], sem_x.at[s])

    def w_copy(j):
        src = (wq_hbm, wk_hbm, wv_hbm, wo_hbm)[j]
        return pltpu.make_async_copy(src.bitcast(i32), wraw.at[j], sem_w.at[j])

    def f_copy(j, c):
        src, dst = ((wg_hbm, wg), (wu_hbm, wu), (wd_hbm, wd))[j]
        off = c * FC if isinstance(c, int) else pl.multiple_of(c * FC, FC)
        return pltpu.make_async_copy(src.bitcast(i32).at[:, pl.ds(off, FC)], dst.at[c],
                                     sem_f.at[j * NFC + c])

    def o_copy(s):
        return pltpu.make_async_copy(obuf.at[s], out32.at[:, pl.ds(s * L, L)], sem_o.at[s])

    x_copy(0).start()
    for j in range(3):
        w_copy(j).start()
    for s in range(1, NSEG):
        x_copy(s).start()
    w_copy(3).start()
    for c in range(NFC):
        for j in range(3):
            f_copy(j, c).start()

    tri[...] = jnp.where(_iota((128, 128), 0) > _iota((128, 128), 1), NEG, 0.0).astype(f32)
    g_row = _rnd(jax.nn.sigmoid(beta_ref[...].astype(f32).reshape(1, H)))
    eye = _iota((H, H), 0) == _iota((H, H), 1)
    g_col = jnp.sum(jnp.where(eye, jnp.broadcast_to(g_row, (H, H)), 0.0), axis=1, keepdims=True)
    g_all = jnp.broadcast_to(g_col, (H, 128))
    gate[...] = g_all
    for g in range(NG):
        gate1[g] = _rnd(1.0 - g_all[GH * g:GH * g + GH])
    for half in range(2):
        r_, c_ = _iota((80, 128), 0), _iota((80, 128), 1)
        first, spare = 8 * half, 72 * (1 - half)
        keep = None
        for j in range(4):
            lo = first + DH * j
            m = _between(c_, lo, lo + DH) & (_between(r_, lo, lo + DH) | (r_ == spare + j))
            keep = m if keep is None else keep | m
        mmask[half] = jnp.where(keep, 1.0, 0.0)
    wr = wr_ref[...].astype(f32).reshape(1, D)
    wvt[DP:DP + 8, :] = _w(jnp.broadcast_to(wr, (16, D)).astype(bf16))
    hbuf[...] = jnp.zeros(hbuf.shape, hbuf.dtype)
    yacc[...] = jnp.zeros(yacc.shape, yacc.dtype)

    def layernorm(s):
        for t in range(L // 128):
            x = _b(xs[s, :, 128 * t:128 * t + 128]).astype(f32)
            mean = jnp.sum(x, axis=0, keepdims=True) * (1.0 / D)
            xc = x - mean
            var = jnp.sum(xc * xc, axis=0, keepdims=True) * (1.0 / D)
            sd = _rnd(jnp.sqrt(_rnd(_rnd(var) + EPS_LN)))
            xn[4 * s + t] = _w((_rnd(x - _rnd(mean)) * (1.0 / sd)).astype(bf16))

    def xn_seg(s):
        return _b(jnp.concatenate([xn[4 * s + t] for t in range(L // 128)], axis=1))

    def put(ref, s, val):
        for g in range(NG):
            ref[NG * s + g] = val[GP * g:GP * g + GP]

    def proj_q(s, w):
        q = _dot(w, xn_seg(s))
        put(qs, s, _w((q * QSCALE).astype(bf16)))
        if s > 0:
            put(pqs, s, _w(_phi(_rnd(q)).astype(bf16)))

    def proj_k(s, w):
        k = _dot(w, xn_seg(s))
        put(kt, s, _w(k.astype(bf16)))
        if s + 1 < NSEG:
            put(pkt, s, _w(_phi(_rnd(k)).astype(bf16)))

    def proj_v(s, w):
        vr = _dot(w, xn_seg(s))
        put(vt, s, _w(vr[0:D].astype(bf16)))
        rs[:, s * L:(s + 1) * L] = _rnd(vr[D:D + 8])

    def key_windows(s):
        for g in range(NG):
            for half in range(2):
                kw[NG * s + g, half] = _w(_b(kt[NG * s + g, 8 * half:8 * half + 64, :]).T)

    def mem_read(s):
        for g in range(NG):
            t = NG * s + g
            for half in range(2):
                w = 2 * g + half
                first, spare = 8 * half, 72 * (1 - half)
                nd = _dot(mz[w][:, 0:80].astype(bf16), _b(pqs[t, 32 * half:32 * half + 40, :]))
                h0 = GH * g + 4 * half
                gw = jnp.concatenate([gate[h0:h0 + 4, :]] * 2, axis=0)
                rden[w] = jnp.tile(gw, (1, L // 128)) / (nd[spare:spare + 8] + 1e-6)
                for rb in range(9):
                    ha, hb = (8 * rb) // DH, (8 * rb + 7) // DH
                    r = jnp.broadcast_to(rden[w, ha:ha + 1, :], (8, L))
                    if ha != hb:
                        r = jnp.where(_iota((8, L), 0) < DH * hb - 8 * rb, r,
                                      jnp.broadcast_to(rden[w, hb:hb + 1, :], (8, L)))
                    row = 72 * half + 8 * rb
                    amem[t, row:row + 8, :] = nd[first + 8 * rb:first + 8 * rb + 8] * r

    def mem_update(s):
        for g in range(NG):
            t = NG * s + g
            for half in range(2):
                w = 2 * g + half
                sp = 36 * (1 - half)
                v = jnp.where(_between(_iota((40, L), 0), sp, sp + 4), ONES2,
                              vt[t, 32 * half:32 * half + 40, :])
                upd = _dot_nt(_b(v), _b(pkt[t, 32 * half:32 * half + 40, :]))
                upd = jnp.where(mmask[half, :, 0:80] > 0, upd, 0.0)
                mz[w, :, 0:80] = upd if s == 0 else mz[w, :, 0:80] + upd

    def route():
        r = rs[...]
        tok = _iota((8, S), 1)
        m1 = jnp.max(r, axis=1, keepdims=True)
        i1 = jnp.min(jnp.where(r == m1, tok, S), axis=1, keepdims=True)
        r2 = jnp.where(tok == i1, -jnp.inf, r)
        m2 = jnp.max(r2, axis=1, keepdims=True)
        i2 = jnp.min(jnp.where((r2 == m2) & (tok != i1), tok, S), axis=1, keepdims=True)
        row = _iota((8, S), 0)
        one8 = jnp.where(((row == 0) & (tok == i1)) | ((row == 1) & (tok == i2)), 1.0, 0.0)
        one = _w(jnp.concatenate([one8, jnp.zeros((8, S), f32)], axis=0).astype(bf16))
        for t in range(S // 128):
            sel[t] = one[:, 128 * t:128 * t + 128]
        rs8 = _rnd(jax.nn.sigmoid(jnp.where(_iota((8, 1), 0) == 0, m1, m2)))
        rsel[...] = jnp.broadcast_to(rs8, (8, 128))
        t1 = jnp.clip(jnp.max(i1) // 128, 0, S // 128 - 1)
        t2 = jnp.clip(jnp.max(i2) // 128, 0, S // 128 - 1)
        xa = _dot_nt(_b(sel[t1]), _b(xn[t1]))
        xb = _dot_nt(_b(sel[t2]), _b(xn[t2]))
        xsel[...] = _w(jnp.where(_iota((16, D), 0) == 0, xa, xb).astype(bf16))

    def ffn_jobs(c_up, c_down):
        jobs = []
        acc = {}

        def down(n):
            n0, n1 = 128 * n, min(128 * n + 128, D)
            yacc[:, n0:n1] += _dot_nt(_b(acc["h"]), _b(wd[c_down, n0 // 2:n1 // 2, :]))

        def up(j, k):
            k0, k1 = 128 * k, min(128 * k + 128, D)
            part = _dot(_b(xsel[:, k0:k1]), _b((wg, wu)[j][c_up, k0 // 2:k1 // 2, :]))
            acc[j] = part if k == 0 else acc[j] + part
            if j == 1 and k1 == D:
                g, u = _rnd(acc[0]), _rnd(acc[1])
                hbuf[...] = _w((_rnd(g * jax.nn.sigmoid(g)) * u).astype(bf16))

        if c_down is not None:
            acc["h"] = hbuf[...]
            jobs += [(down, n) for n in range(5)]
        if c_up is not None:
            jobs += [(up, j, k) for j in range(2) for k in range(5)]
        return jobs

    def ffn_finish():
        y = _rnd(_rnd(yacc[...]) * jnp.tile(rsel[:, 0:1], (2, 1)))
        ypad = jnp.concatenate([y, jnp.zeros((112, D), f32)], axis=0)
        wot[:, D:D + 16] = _w(ypad.T[:, 0:16].astype(bf16))

    def att_step(tq, s_w, m_w, tp, s_r, m_r, extra=()):
        qm, mx, acc = {}, {}, {}

        def scores(h, i, j):
            half = h // 4
            if j == 0:
                prow = _iota((64, 128), 0) + 8 * half
                q = qs[tq, 8 * half:8 * half + 64, 128 * i:128 * i + 128]
                qm[h] = _b(jnp.where(_between(prow, 9 * h, 9 * h + 9), q, 0))
            sc = _dot(_b(kw[tq, half, 64 * j:64 * j + 64, :]), qm[h])
            if j == i:
                sc = sc + tri[...]
            mm = jnp.max(sc.reshape(16, 8, 128), axis=0)
            mx[h] = mm if j == 0 else jnp.maximum(mx[h], mm)
            if j == i:
                m_w[h, i] = jnp.broadcast_to(jnp.max(mx[h], axis=0, keepdims=True), (8, 128))
            s_w[h, i * (i + 1) // 2 + j] = sc

        def values(h, i, j):
            sc = s_r[h, i * (i + 1) // 2 + j].reshape(16, 8, 128)
            p = jnp.exp2(sc - m_r[h, i][None]).reshape(128, 128).astype(bf16)
            a = (9 * h) // 8
            v = jnp.where(_between(_iota((16, 128), 0) + 8 * a, 9 * h, 9 * h + 9),
                          vt[tp, 8 * a:8 * a + 16, 128 * j:128 * j + 128], ONES2)
            o = _dot(_b(v), p)
            acc[h] = o if j == 0 else acc[h] + o
            if j < i:
                return
            o = acc[h]
            r0 = 8 if DH * h - 16 * a >= 8 else 0
            den = o[0:8] if r0 else o[24:32]
            g1 = jnp.broadcast_to(gate1[tp % NG, h:h + 1, :], (8, 128))
            scale = g1 / den
            for rb in range(3):
                lo = 16 * a + r0 + 8 * rb
                val = o[r0 + 8 * rb:r0 + 8 * rb + 8] * scale
                dst = adot.at[tp, lo:lo + 8, 128 * i:128 * i + 128]
                if lo >= DH * h and lo + 8 <= DH * h + DH:
                    dst[...] = val
                else:
                    pltpu.store(dst, val,
                                mask=_between(_iota((8, 128), 0) + lo, DH * h, DH * h + DH))

        extra = list(extra)
        units = [(hq, i, j) for hq in (0, 4) for i in range(4) for j in range(i + 1)]
        for n, (hq, i, j) in enumerate(units):
            if tq is not None:
                for h in range(hq, hq + 4):
                    scores(h, i, j)
            if tp is not None:
                for h in range(hq, hq + 4):
                    values(h, i, j)
            while extra and len(extra) * len(units) > (len(units) - 1 - n) * extra_total[0]:
                fn, *args = extra.pop(0)
                fn(*args)

    extra_total = [0]

    def run_step(tq, tp, bufs, extra=()):
        extra_total[0] = len(extra)
        (s_w, m_w), (s_r, m_r) = bufs
        att_step(tq, s_w, m_w, tp, s_r, m_r, extra)

    def out_proj(s):
        o = jnp.concatenate([adot[NG * s + g] for g in range(NG)], axis=0)
        if s > 0:
            o = o + jnp.concatenate([amem[NG * s + g] for g in range(NG)], axis=0)
        one = jnp.concatenate([sel[4 * s + t] for t in range(L // 128)], axis=1)
        rhs = _b(jnp.concatenate([_w(o.astype(bf16)), one], axis=0))
        res = _dot(_b(wot[:, 0:D + 16]), rhs)
        res = res + (_b(xs[s]).astype(f32) + xn_seg(s).astype(f32))
        obuf[s] = _w(res.astype(bf16))

    even, odd = ((s_a, m_a), (s_b, m_b)), ((s_b, m_b), (s_a, m_a))

    with jax.named_scope("w0"):
        x_copy(0).wait()
    layernorm(0)
    with jax.named_scope("w1"):
        w_copy(0).wait()
    w = _b(wraw[0]).T
    wqt[...] = _w(w)
    proj_q(0, w)
    with jax.named_scope("w2"):
        w_copy(1).wait()
    w = _b(wraw[1]).T
    wkt[...] = _w(w)
    proj_k(0, w)
    with jax.named_scope("w3"):
        w_copy(2).wait()
        x_copy(1).wait()
    w = _w(_b(wraw[2]).T)
    wvt[0:DP, :] = w
    proj_v(0, _b(jnp.concatenate([w, wvt[DP:DP + 8, :]], axis=0)))
    layernorm(1)
    for s in range(1, NSEG):
        with jax.named_scope("w4"):
            if s + 1 < NSEG:
                x_copy(s + 1).wait()
            else:
                w_copy(3).wait()
        proj_q(s, _b(wqt[...]))
        if s > 1:
            mem_read(s - 1)
        proj_k(s, _b(wkt[...]))
        mem_update(s - 1)
        proj_v(s, _b(wvt[...]))
        key_windows(s - 1)
        if s + 1 < NSEG:
            layernorm(s + 1)
        else:
            wot[:, 0:D] = _w(_b(wraw[3]).T)

    with jax.named_scope("w5"):
        for j in range(3):
            f_copy(j, 0).wait()
    run_step(0, None, even)
    key_windows(NSEG - 1)
    mem_read(NSEG - 1)
    route()

    def ffn_pair(n, carry):
        c = 2 * n
        for j in range(3):
            f_copy(j, c + 1).wait()
            f_copy(j, c + 2).wait()
        run_step(c + 1, c, odd, ffn_jobs(c, jnp.maximum(c - 1, 0)))
        run_step(c + 2, c + 1, even, ffn_jobs(c + 1, c))
        return carry

    with jax.named_scope("loop1"):
        lax.fori_loop(0, 4, ffn_pair, 0)
    run_step(9, 8, odd, ffn_jobs(8, 7))

    def plain_pair(n, carry):
        c = 2 * n + 1

        @pl.when(n == 5)
        def _():
            for fn, *args in ffn_jobs(None, NFC - 1):
                fn(*args)
            ffn_finish()

        run_step(c + 1, c, even)
        run_step(c + 2, c + 1, odd)
        return carry

    with jax.named_scope("loop2"):
        lax.fori_loop(4, 7, plain_pair, 0)

    run_step(None, NSTEP - 1, even, [(out_proj, 0)])
    o_copy(0).start()
    for s in range(1, NSEG):
        out_proj(s)
        o_copy(s).start()
    with jax.named_scope("w6"):
        for s in range(NSEG):
            o_copy(s).wait()


@jax.jit
def pallas_parallel_sum__memory_aug_infini_attn__moe_arch_mod__prompt_kernel(
    A_x, A_wq, A_wk, A_wv, A_wo, A_beta, B_x, B_w_r, B_w_gate, B_w_up, B_w_down,
):
    hbm = pl.BlockSpec(memory_space=pl.ANY)
    vmem = pl.BlockSpec(memory_space=pltpu.VMEM)
    out = pl.pallas_call(
        _kernel,
        out_shape=jax.ShapeDtypeStruct((D, S), bf16),
        in_specs=[hbm, hbm, hbm, hbm, hbm, vmem, vmem, hbm, hbm, hbm],
        out_specs=hbm,
        scratch_shapes=[
            pltpu.VMEM((NSEG, DP, L), i32),
            pltpu.VMEM((S // 128, DP, 128), i32),
            pltpu.VMEM((4, DP, D), i32),
            pltpu.VMEM((DP, D), i32),
            pltpu.VMEM((DP, D), i32),
            pltpu.VMEM((DP + 8, D), i32),
            pltpu.VMEM((DP, 640), i32),
            pltpu.VMEM((NSTEP, GP, L), i32),
            pltpu.VMEM((NSTEP, GP, L), i32),
            pltpu.VMEM((NSTEP, GP, L), i32),
            pltpu.VMEM((NSTEP, GP, L), i32),
            pltpu.VMEM((NSTEP, GP, L), i32),
            pltpu.VMEM((NSTEP, 2, L // 2, 128), i32),
            pltpu.VMEM((NSTEP, GR, L), f32),
            pltpu.VMEM((NSTEP, GR, L), f32),
            pltpu.VMEM((2 * NG, 80, 128), f32),
            pltpu.VMEM((2, 80, 128), f32),
            pltpu.VMEM((NFC, DP, FC), i32),
            pltpu.VMEM((NFC, DP, FC), i32),
            pltpu.VMEM((NFC, DP, FC), i32),
            pltpu.VMEM((NSEG, DP, L), i32),
            pltpu.VMEM((8, S), f32),
            pltpu.VMEM((128, 128), f32),
            pltpu.VMEM((H, 128), f32),
            pltpu.VMEM((NG, GH, 128), f32),
            pltpu.VMEM((2 * NG, 8, L), f32),
            pltpu.VMEM((S // 128, 8, 128), i32),
            pltpu.VMEM((8, D), i32),
            pltpu.VMEM((8, 128), f32),
            pltpu.VMEM((8, FC), i32),
            pltpu.VMEM((16, D), f32),
            pltpu.VMEM((GH, 10, 128, 128), f32),
            pltpu.VMEM((GH, 10, 128, 128), f32),
            pltpu.VMEM((GH, 4, 8, 128), f32),
            pltpu.VMEM((GH, 4, 8, 128), f32),
            pltpu.SemaphoreType.DMA((NSEG,)),
            pltpu.SemaphoreType.DMA((4,)),
            pltpu.SemaphoreType.DMA((3 * NFC,)),
            pltpu.SemaphoreType.DMA((NSEG,)),
        ],
        compiler_params=pltpu.CompilerParams(vmem_limit_bytes=100 * 1024 * 1024),
        name="infini_mod",
    )(A_x[0].T, A_wq, A_wk, A_wv, A_wo, A_beta, B_w_r, B_w_gate, B_w_up, B_w_down.T)
    return out.T[None]
```

```python
import functools
import math

import jax
import jax.numpy as jnp
import numpy as np
from jax import lax
import jax.experimental.pallas as pl
import jax.experimental.pallas.tpu as pltpu

S, D, H, DH, NSEG, L, F = 2048, 576, 32, 18, 4, 512, 4608
DP = D // 2
GH, GR, GP = 8, 144, 72
NG = H // GH
NSTEP = NSEG * NG
NT = S // 128
FC = 512
NFC = F // FC
LOG2E = math.log2(math.e)
QSCALE = DH ** -0.5 * LOG2E
NEG = -1e9 * LOG2E
EPS_LN = float(np.asarray(1e-5, dtype=jnp.bfloat16))
IN_CHUNKS = ((0, 1), (1, 2), (2, 3), (3, 4), (4, 8), (8, 16))
OUT_CHUNKS = ((0, 4), (4, 8), (8, 12), (12, 14), (14, 15), (15, 16))
ONES2 = np.int32(0x3F803F80)
WQ_SPLIT = 384
Q_ORDER, P_ORDER, P_SKIP = (0, 1, 2, 3), (3, 2, 1, 0), 0

count = [0]
f32, bf16, i32 = jnp.float32, jnp.bfloat16, jnp.int32


def _b(x):
    return pltpu.bitcast(x, bf16)


def _w(x):
    return pltpu.bitcast(x, i32)


def _rnd(x):
    return x.astype(bf16).astype(f32)


def _phi(t):
    return jnp.where(t > 0, t + 1.0, jnp.exp(t))


def _dot(a, b):
    return jnp.dot(a, b, preferred_element_type=f32)


def _dot_nt(a, b):
    return lax.dot_general(a, b, (((1,), (1,)), ((), ())), preferred_element_type=f32)


def _iota(shape, dim):
    return lax.broadcasted_iota(i32, shape, dim)


def _between(x, lo, hi):
    return (x >= lo) & (x < hi)


def _rotate(x, quarters):
    if quarters % 4 == 0:
        return x
    tiles = [pltpu.roll(x[:, c:c + 128], 32 * (quarters % 4), 1)
             for c in range(0, x.shape[1], 128)]
    return tiles[0] if len(tiles) == 1 else jnp.concatenate(tiles, axis=1)


def _head_rows(h):
    return 9 * h // 8 * 8, 9 * h // 8 * 8 + 8


def _interleave(main, extra):
    done = 0
    for n, job in enumerate(main):
        job()
        while done * len(main) < (n + 1) * len(extra):
            extra[done]()
            done += 1


def _job(fn, *args, **kw):
    return lambda: fn(*args, **kw)


def _compute(x_hbm, wq_hbm, wk_hbm, wv_hbm, wo_hbm, beta_hbm, wr_hbm, wg_hbm, wu_hbm, wd_hbm,
            obuf,
            beta_v, wr_v, xs, xn, wraw, wq0, wq1, wqt, wkt, wvt, wot, wrt, qs, qsh, pqs, kt, pkt, vt, vw, kw, amem, adot,
            ot, mz, mmask, wg, wu, wd, rs, tri, gate, gate1, rden, sel, xsel, rsel, gbuf, hbuf,
            s_a, s_b, m_a, m_b, oacc,
            o_copy, sem_x, sem_w, sem_f):
    x32 = x_hbm.bitcast(i32)

    def x_copy(c):
        lo, hi = IN_CHUNKS[c]
        cols = pl.ds(128 * lo, 128 * (hi - lo))
        return pltpu.make_async_copy(x32.at[:, cols], xs.at[:, cols], sem_x.at[c])

    def wq_copy(c):
        cols = pl.ds(0, WQ_SPLIT) if c == 0 else pl.ds(WQ_SPLIT, D - WQ_SPLIT)
        return pltpu.make_async_copy(wq_hbm.bitcast(i32).at[:, cols], (wq0, wq1)[c],
                                     sem_w.at[0 if c == 0 else 6])

    def w_copy(j):
        if j >= 4:
            src, dst = ((beta_hbm, beta_v), (wr_hbm, wr_v))[j - 4]
            return pltpu.make_async_copy(src, dst, sem_w.at[j])
        src = (wq_hbm, wk_hbm, wv_hbm, wo_hbm)[j]
        return pltpu.make_async_copy(src.bitcast(i32), wraw.at[j], sem_w.at[j])

    def f_copy(j):
        src, dst = ((wg_hbm, wg), (wu_hbm, wu), (wd_hbm, wd))[j]
        return pltpu.make_async_copy(src.bitcast(i32), dst, sem_f.at[j])

    for c in (x_copy(0), wq_copy(0), x_copy(1), x_copy(2), x_copy(3), wq_copy(1), w_copy(4),
              w_copy(5), w_copy(1), w_copy(2), x_copy(4), x_copy(5), w_copy(3)):
        c.start()
    for j in range(3):
        f_copy(j).start()

    def pin(i, carry):
        for ref in (s_a, s_b, m_a, m_b):
            ref[i, 0, 0:8, :] = jnp.zeros((8, 128), f32)
        for ref in (qs, qsh, pqs, kt, pkt, vt, vw, amem, adot, ot, mz, tri, rden, oacc):
            ref[i, 0:8, 0:128] = jnp.zeros((8, 128), ref.dtype)
        kw[i, 0, 0:8, :] = jnp.zeros((8, 128), i32)
        for ref in (wqt, wkt, wvt, wot, hbuf, gbuf):
            ref[0:8, pl.ds(pl.multiple_of(128 * i, 128), 128)] = jnp.zeros((8, 128), ref.dtype)
        return carry

    lax.fori_loop(0, 2, pin, 0)

    key, lane = _iota((32, 128), 0), _iota((32, 128), 1)
    for a in range(4):
        tri[a] = jnp.where(key > (lane + 128 - 32 * a) % 128, NEG, 0.0)
    tri[4] = jnp.where(key > lane % 32, NEG, 0.0)
    for half in range(2):
        r_, c_ = _iota((80, 128), 0), _iota((80, 128), 1)
        first, spare = 8 * half, 72 * (1 - half)
        keep = None
        for j in range(4):
            lo = first + DH * j
            m = _between(c_, lo, lo + DH) & (_between(r_, lo, lo + DH) | (r_ == spare + j))
            keep = m if keep is None else keep | m
        mmask[half] = jnp.where(keep, 1.0, 0.0)

    def small_inputs():
        g_row = _rnd(jax.nn.sigmoid(beta_v[...].astype(f32).reshape(1, H)))
        eye = _iota((H, H), 0) == _iota((H, H), 1)
        g_col = jnp.sum(jnp.where(eye, jnp.broadcast_to(g_row, (H, H)), 0.0), axis=1,
                        keepdims=True)
        g_all = jnp.broadcast_to(g_col, (H, 128))
        gate[...] = g_all
        gate1[...] = _rnd(1.0 - g_all)
        wr = wr_v[...].astype(f32).reshape(1, D)
        wrt[...] = _w(jnp.broadcast_to(wr, (16, D)).astype(bf16))

    def layernorm(t):
        x = _b(xs[:, 128 * t:128 * t + 128]).astype(f32)
        mean = jnp.sum(x, axis=0, keepdims=True) * (1.0 / D)
        mean_r = _rnd(mean)
        xc = x - mean_r
        shift = mean - mean_r
        var = jnp.sum(xc * xc, axis=0, keepdims=True) * (1.0 / D) - shift * shift
        sd = _rnd(jnp.sqrt(_rnd(_rnd(jnp.maximum(var, 0.0)) + EPS_LN)))
        xn[t] = _w((_rnd(xc) * (1.0 / sd)).astype(bf16))

    def layernorm_now(t):
        def rows(r):
            return _b(xs[r:r + 16, 128 * t:128 * t + 128]).astype(f32)

        def average(parts):
            return jnp.sum(functools.reduce(jnp.add, parts), axis=0, keepdims=True) * (1.0 / D)

        mean = average(rows(r) for r in range(0, DP, 16))
        mean_r = _rnd(mean)

        def square(r):
            xc = rows(r) - mean_r
            xn[t, r:r + 16] = _w(xc.astype(bf16))
            return xc * xc

        shift = mean - mean_r
        var = average(square(r) for r in range(0, DP, 16)) - shift * shift
        inv = 1.0 / _rnd(jnp.sqrt(_rnd(_rnd(jnp.maximum(var, 0.0)) + EPS_LN)))
        for r in range(0, DP, 16):
            xn[t, r:r + 16] = _w((_b(xn[t, r:r + 16]).astype(f32) * inv).astype(bf16))

    def score_tokens(t):
        r = _dot(_b(wrt[...]), _b(xn[t]))
        rs[:, 128 * t:128 * t + 128] = _rnd(r[0:8])

    def tiles(ref, lo, hi):
        return jnp.concatenate([ref[t] for t in range(lo, hi)], axis=1)

    def proj(kind, s, g, lo=0, hi=4, w=None, fence=None):
        t, cols, n = NG * s + g, slice(128 * lo, 128 * hi), 128 * (hi - lo)
        if w is None:
            w = {"q": wqt, "k": wkt, "v": wvt}[kind][GP * g:GP * g + GP, :]
        y = _dot(_b(w), _b(tiles(xn, 4 * s + lo, 4 * s + hi)))
        if fence is not None:
            fence()
        if kind == "q":
            q = _w((y * QSCALE).astype(bf16))
            turned = {(h, r): jnp.where(_between(_iota((8, n), 0) + r, 9 * h, 9 * h + 9),
                                        _rotate(q[r:r + 8], h), 0)
                      for h in range(GH) for r in _head_rows(h)}
            for (h, r), val in turned.items():
                qs[t, 16 * h + r - _head_rows(h)[0]:16 * h + r - _head_rows(h)[0] + 8, cols] = val
            quarter = _iota((8, n), 1) // 32 % 4
            for hq in (0, 4):
                for u in (1, 2, 3):
                    for r in range(8 * hq, 8 * hq + 40, 8):
                        val = 0
                        for h in range(hq, hq + 4):
                            if (h, r) in turned:
                                val = jnp.where(quarter == (u + h) % 4, turned[h, r], val)
                        row = 40 * (3 * (hq // 4) + u - 1) + r - 8 * hq
                        qsh[t, row:row + 8, cols] = val
            if s > 0:
                pqs[t, :, cols] = _w(_phi(y).astype(bf16))
        elif kind == "k":
            kt[t, :, cols] = _w(y.astype(bf16))
            if s + 1 < NSEG:
                pkt[t, :, cols] = _w(_phi(y).astype(bf16))
        else:
            if s + 1 < NSEG:
                vt[t, :, cols] = _w(y.astype(bf16))
            for h in range(GH):
                base = (DH * h) // 8 * 8
                vw[t, 24 * h:24 * h + 24, cols] = jnp.where(
                    _between(_iota((24, n), 0) + base, DH * h, DH * h + DH), y[base:base + 24], 1.0)

    def key_window(t, half):
        kw[t, half] = _w(_b(kt[t, 8 * half:8 * half + 64, :]).T)

    def mem_read(t, half):
        w = 2 * (t % NG) + half
        first, spare = 8 * half, 72 * (1 - half)
        nd = _dot(mz[w, :, 0:80].astype(bf16), _b(pqs[t, 32 * half:32 * half + 40, :]))
        gw = jnp.concatenate([gate[4 * w:4 * w + 4, :]] * 2, axis=0)
        rden[w] = jnp.tile(gw, (1, L // 128)) / (nd[spare:spare + 8] + 1e-6)
        for rb in range(9):
            ha, hb = (8 * rb) // DH, (8 * rb + 7) // DH
            r = jnp.broadcast_to(rden[w, ha:ha + 1, :], (8, L))
            if ha != hb:
                r = jnp.where(_iota((8, L), 0) < DH * hb - 8 * rb, r,
                              jnp.broadcast_to(rden[w, hb:hb + 1, :], (8, L)))
            row = 72 * half + 8 * rb
            amem[t, row:row + 8, :] = nd[first + 8 * rb:first + 8 * rb + 8] * r

    def mem_update(t, half):
        w = 2 * (t % NG) + half
        spare = 36 * (1 - half)
        v = jnp.where(_between(_iota((40, L), 0), spare, spare + 4), ONES2,
                      vt[t, 32 * half:32 * half + 40, :])
        upd = _dot_nt(_b(v), _b(pkt[t, 32 * half:32 * half + 40, :]))
        upd = jnp.where(mmask[half, :, 0:80] > 0, upd, 0.0)
        mz[w, :, 0:80] = upd if t < NG else mz[w, :, 0:80] + upd

    def post_jobs(t):
        jobs = [_job(key_window, t, half) for half in range(2)]
        if t >= NG:
            jobs += [_job(mem_read, t, half) for half in range(2)]
        if t < NSTEP - NG:
            jobs += [_job(mem_update, t, half) for half in range(2)]
        return jobs

    routed = {}

    def route():
        r = rs[...]
        tok = _iota((8, S), 1)
        m1 = jnp.max(r, axis=1, keepdims=True)
        i1 = jnp.min(jnp.where(r == m1, tok, S), axis=1, keepdims=True)
        r2 = jnp.where(tok == i1, -jnp.inf, r)
        m2 = jnp.max(r2, axis=1, keepdims=True)
        i2 = jnp.min(jnp.where((r2 == m2) & (tok != i1), tok, S), axis=1, keepdims=True)
        row = _iota((8, S), 0)
        one8 = jnp.where(((row == 0) & (tok == i1)) | ((row == 1) & (tok == i2)), 1.0, 0.0)
        one = _w(jnp.concatenate([one8, jnp.zeros((8, S), f32)], axis=0).astype(bf16))
        for t in range(NT):
            sel[t] = one[:, 128 * t:128 * t + 128]
        rs8 = _rnd(jax.nn.sigmoid(jnp.where(_iota((8, 1), 0) == 0, m1, m2)))
        rsel[...] = jnp.broadcast_to(rs8, (8, 128))
        routed["tiles"] = [jnp.clip(jnp.max(i) // 128, 0, NT - 1) for i in (i1, i2)]

    def gather():
        xa, xb = [_dot_nt(_b(sel[t]), _b(xn[t])) for t in routed["tiles"]]
        xsel[...] = jnp.where(_iota((8, D), 0) == 0, xa[0:8], xb[0:8])

    ffn = {}

    def ffn_up(c, j, k):
        k0, k1 = 128 * k, min(128 * k + 128, D)
        w = _b((wg, wu)[j][k0 // 2:k1 // 2, FC * c:FC * c + FC]).astype(f32)
        part = _dot(xsel[:, k0:k1], w)
        ffn[j] = part if k == 0 else ffn[j] + part
        if k1 == D and j == 0:
            g = _rnd(ffn[0])
            gbuf[:, FC * c:FC * c + FC] = _rnd(g * jax.nn.sigmoid(g))
        elif k1 == D:
            hbuf[:, FC * c:FC * c + FC] = _rnd(gbuf[:, FC * c:FC * c + FC] * _rnd(ffn[1]))

    def ffn_down(n, c):
        n0, n1 = 128 * n, min(128 * n + 128, D)
        w = _b(wd[n0 // 2:n1 // 2, FC * c:FC * c + FC]).astype(f32)
        part = _dot_nt(hbuf[:, FC * c:FC * c + FC], w)
        ffn["y", n] = part if c == 0 else ffn["y", n] + part

    def ffn_finish():
        y = jnp.concatenate([ffn["y", n] for n in range(5)], axis=1)
        y = _rnd(_rnd(y) * rsel[:, 0:1])
        ypad = jnp.concatenate([y, jnp.zeros((120, D), f32)], axis=0)
        wot[:, D:D + 16] = _w(ypad.T[:, 0:16].astype(bf16))

    def att_jobs(tq, tp):
        s_w, m_w = (s_a, m_a) if (tq if tp is None else tp + 1) % 2 == 0 else (s_b, m_b)
        s_r, m_r = (s_b, m_b) if s_w is s_a else (s_a, m_a)
        mx, acc = {}, {}

        def keys(hq, lo, hi):
            return _b(kw[tq, hq // 4, lo // 2:hi // 2, :])

        def padded(q, first):
            before, after = ([jnp.zeros((n, 128), i32)] if n else []
                             for n in (first, 64 - first - q.shape[0]))
            return _b(jnp.concatenate(before + [q] + after, axis=0))

        def queries(hq, i, h):
            return padded(qs[tq, 16 * h:16 * h + 16, 128 * i:128 * i + 128],
                          _head_rows(h)[0] - 2 * hq)

        def shared_queries(hq, i, u):
            row = 40 * (3 * (hq // 4) + u - 1)
            return padded(qsh[tq, row:row + 40, 128 * i:128 * i + 128], 6 * hq)

        def vmax(sc):
            return jnp.max(sc.reshape(-1, 8, 128), axis=0)

        def scores(hq, i, j):
            full = 128 if i > 0 else 0
            part = 32 if j >= i - 1 else 0
            tile = i * (i + 1) // 2
            for h in range(hq, hq + 4):
                sc = _dot(keys(hq, 128 * j, 128 * j + full + part), queries(hq, i, h))
                ms = [mx[h]] if j > 0 else []
                if full:
                    s_w[h, tile + j] = sc[0:full]
                    ms.append(vmax(sc[0:full]))
                if part:
                    d = sc[full:] + tri[h - hq]
                    s_w[h, tile + i, 0:32] = d
                    ms.append(vmax(d))
                mx[h] = functools.reduce(jnp.maximum, ms)

        def shared_scores(hq, i):
            quarter = _iota((8, 128), 1) // 32
            for u in (3, 2, 1):
                sc = _dot(keys(hq, 128 * i + 32, 128 * i + 32 * u + 32),
                          shared_queries(hq, i, u))
                d = sc[32 * u - 32:] + tri[4]
                sc = d if u == 1 else jnp.concatenate([sc[0:32 * u - 32], d], axis=0)
                s_w[hq + u, i * (i + 1) // 2 + i, 32:32 * u + 32] = sc
                mu = vmax(sc)
                for a in range(4):
                    mx[hq + a] = jnp.where(quarter == (u + a) % 4,
                                           jnp.maximum(mx[hq + a], mu), mx[hq + a])
            for h in range(hq, hq + 4):
                m_w[h, i] = jnp.broadcast_to(jnp.max(mx[h], axis=0, keepdims=True), (8, 128))

        def weights(sc, m):
            return jnp.exp2(sc.reshape(-1, 8, 128) - m[None]).reshape(sc.shape)

        def values(hq, i, j):
            tile = i * (i + 1) // 2 + j
            shared = {}
            if j == i:
                for u in (1, 2, 3):
                    m = m_r[hq + (-u) % 4, i]
                    for p in range(1, 4):
                        m = jnp.where(_iota((8, 128), 1) // 32 == p, m_r[hq + (p - u) % 4, i], m)
                    shared[u] = weights(s_r[hq + u, tile, 32:32 * u + 32], m)
            for h in range(hq, hq + 4):
                if j < i:
                    p = weights(s_r[h, tile], m_r[h, i])
                else:
                    parts = [weights(s_r[h, tile, 0:32], m_r[h, i])]
                    for kq in (1, 2, 3):
                        x = 0.0
                        for u in range(kq, 4):
                            x = jnp.where(_iota((32, 128), 1) // 32 == (u + h) % 4,
                                          shared[u][32 * kq - 32:32 * kq], x)
                        parts.append(x)
                    p = jnp.concatenate(parts, axis=0)
                base = (DH * h) // 8 * 8
                o = _dot(vw[tp, 24 * h:24 * h + 24, 128 * j:128 * j + 128], p)
                if j > 0:
                    o = (oacc[h] if j == 1 else acc[h]) + o
                if j < i:
                    if j == 0:
                        oacc[h] = o
                    acc[h] = o
                    continue
                free = 0 if DH * h > base else 23
                hg = GH * (tp % NG) + h
                scale = (jnp.broadcast_to(gate1[hg:hg + 1, :], (8, 128))
                         * pltpu.reciprocal(jnp.broadcast_to(o[free:free + 1], (8, 128)),
                                            approx=True))
                for lo in range(base, base + 24, 8):
                    val = _rotate(o[lo - base:lo - base + 8] * scale, -h)
                    dst = adot.at[tp, lo:lo + 8, 128 * i:128 * i + 128]
                    if lo >= DH * h and lo + 8 <= DH * h + DH:
                        dst[...] = val
                    else:
                        pltpu.store(dst, val,
                                    mask=_between(_iota((8, 128), 0) + lo, DH * h, DH * h + DH))

        jobs = []
        for hq in (0, 4):
            first, second = [], []
            for i in Q_ORDER:
                first += [(_job(scores, hq, i, j), i > 0) for j in range(max(i, 1))]
                first.append((_job(shared_scores, hq, i), False))
            for i in P_ORDER:
                second += [(_job(values, hq, i, j), False) for j in range(i + 1)]
            second.insert(P_SKIP, None)
            for a, b in zip(first, second):
                if tq is not None:
                    jobs.append(a)
                if tp is not None and b is not None:
                    jobs.append(b)
        return jobs

    def pack_heads(t):
        o = adot[t] if t < NG else adot[t] + amem[t]
        o = _w(o.astype(bf16))
        for c in range(4):
            ot[4 * (t // NG) + c, GP * (t % NG):GP * (t % NG) + GP] = o[:, 128 * c:128 * c + 128]

    def out_proj(c, r0, r1, fence=None):
        lo, hi = OUT_CHUNKS[c]
        rhs = jnp.concatenate([tiles(ot, lo, hi), tiles(sel, lo, hi)], axis=0)
        y = _dot(_b(wot[r0:r1, 0:D + 16]), _b(rhs))
        if fence is not None:
            fence()
        x = xs[r0:r1, 128 * lo:128 * hi]
        xnc = jnp.concatenate([xn[t, r0:r1] for t in range(lo, hi)], axis=1)
        y = y + (_b(x).astype(f32) + _b(xnc).astype(f32))
        obuf[r0:r1, 128 * lo:128 * hi] = _w(y.astype(bf16))

    def out_jobs(c):
        step = GP
        return [_job(out_proj, c, r, r + step,
                     fence=(lambda: o_copy(c - 1).start()) if c > 0 and r == 0 else None)
                for r in range(0, DP, step)]

    def waits(*copies):
        def run():
            count[0] += 1
            if True:
                for c in copies:
                    c.wait()
        return run

    def transposed(j, dst):
        w = _w(_b(wraw[j]).T)
        dst[0:DP, 0:D] = w
        return w

    waits(x_copy(0))()
    layernorm_now(0)
    waits(wq_copy(0))()
    w = _w(_b(wq0[...]).T)
    wqt[0:WQ_SPLIT // 2, :] = w
    proj("q", 0, 0, 0, 1, w=w[0:GP])
    proj("q", 0, 1, 0, 1, w=w[GP:2 * GP], fence=waits(x_copy(1), x_copy(2)))
    for t in (1, 2):
        layernorm_now(t)
        proj("q", 0, 0, t, t + 1)
        proj("q", 0, 1, t, t + 1, fence=(
            waits(x_copy(3), wq_copy(1), w_copy(4), w_copy(5)) if t == 2 else None))
    wqt[WQ_SPLIT // 2:, :] = _w(_b(wq1[...]).T)
    layernorm_now(3)
    small_inputs()
    proj("q", 0, 2, 0, 3)
    for g in range(3):
        proj("q", 0, g, 3, 4, fence=waits(w_copy(1)) if g == 2 else None)
    transposed(1, wkt)
    proj("q", 0, 3)
    proj("k", 0, 0)
    score_tokens(0)
    proj("k", 0, 1)
    score_tokens(1)
    proj("k", 0, 2, fence=waits(w_copy(2)))
    transposed(2, wvt)
    score_tokens(2)
    proj("k", 0, 3, fence=waits(x_copy(4)))
    score_tokens(3)
    for g in range(NG):
        layernorm(4 + g)
        proj("v", 0, g)
        score_tokens(4 + g)
    for s in range(1, NSEG):
        fence = waits(x_copy(5), w_copy(3)) if s == 1 else None
        for g in range(NG):
            t = NG * s + g
            extra = post_jobs(t - 1) if t > NG else sum((post_jobs(u) for u in range(NG)), [])
            if s + 1 < NSEG:
                extra.insert(1, _job(layernorm, t + NG))
                extra.append(_job(score_tokens, t + NG))
            else:
                extra.insert(1, (_job(transposed, 3, wot), route, gather, lambda: None)[g])
            _interleave([_job(proj, "q", s, g, fence=fence if g == 0 else None),
                         _job(proj, "k", s, g), _job(proj, "v", s, g)], extra)

    _interleave([job for job, _ in att_jobs(0, None)], post_jobs(NSTEP - 1))
    ffn_work = []
    for c in range(NFC + 1):
        for k in range(5):
            if c < NFC:
                ffn_work += [_job(ffn_up, c, *divmod(2 * k + n, 5)) for n in range(2)]
            if c > 0:
                ffn_work.append(_job(ffn_down, k, c - 1))
    ffn_work += [ffn_finish]
    per_step = -(-len(ffn_work) // (NSTEP - 3))
    for t in range(1, NSTEP):
        extra = ffn_work[per_step * (t - 2):per_step * (t - 1)] if t > 1 else []
        if t == 2:
            waits(f_copy(0), f_copy(1), f_copy(2))()
        if t >= 2:
            pack_heads(t - 2)
        jobs = att_jobs(t, t - 1)
        rooms, seen, done = sum(roomy for _, roomy in jobs), 0, 0
        for job, roomy in jobs:
            job()
            seen += roomy
            if roomy and done < len(extra) and done * rooms < seen * len(extra):
                extra[done]()
                done += 1

    _interleave(out_jobs(0), [_job(pack_heads, NSTEP - 2)]
                + [job for job, _ in att_jobs(None, NSTEP - 1)])
    _interleave(out_jobs(1), [_job(pack_heads, NSTEP - 1)])
    for c in range(2, len(OUT_CHUNKS)):
        _interleave(out_jobs(c), [])
    o_copy(len(OUT_CHUNKS) - 1).start()


def _kernel(*refs):
    inputs, (out_hbm, sem_o, obuf), scratch = refs[:10], refs[10:13], refs[13:]

    def o_copy(c):
        lo, hi = OUT_CHUNKS[c]
        cols = pl.ds(128 * lo, 128 * (hi - lo))
        return pltpu.make_async_copy(obuf.at[:, cols], out_hbm.bitcast(i32).at[:, cols], sem_o)

    pl.run_scoped(functools.partial(_compute, *inputs, obuf, *scratch, o_copy),
                  pltpu.SemaphoreType.DMA((len(IN_CHUNKS),)), pltpu.SemaphoreType.DMA((7,)),
                  pltpu.SemaphoreType.DMA((3,)))
    if True:
        for c in range(len(OUT_CHUNKS)):
            o_copy(c).wait()


@jax.jit
def pallas_parallel_sum__memory_aug_infini_attn__moe_arch_mod__prompt_kernel(
    A_x, A_wq, A_wk, A_wv, A_wo, A_beta, B_x, B_w_r, B_w_gate, B_w_up, B_w_down,
):
    hbm = pl.BlockSpec(memory_space=pl.ANY)
    out = pl.pallas_call(
        _kernel,
        out_shape=jax.ShapeDtypeStruct((D, S), bf16),
        in_specs=[hbm] * 10,
        out_specs=hbm,
        scratch_shapes=[
            pltpu.SemaphoreType.DMA(()),
            pltpu.VMEM((DP, S), i32),
            pltpu.VMEM((H,), bf16),
            pltpu.VMEM((D,), bf16),
            pltpu.VMEM((DP, S), i32),
            pltpu.VMEM((NT, DP, 128), i32),
            pltpu.VMEM((4, DP, D), i32),
            pltpu.VMEM((DP, WQ_SPLIT), i32),
            pltpu.VMEM((DP, D - WQ_SPLIT), i32),
            pltpu.VMEM((DP, D), i32),
            pltpu.VMEM((DP, D), i32),
            pltpu.VMEM((DP, D), i32),
            pltpu.VMEM((DP, 640), i32),
            pltpu.VMEM((8, D), i32),
            pltpu.VMEM((NSTEP, 16 * GH, L), i32),
            pltpu.VMEM((NSTEP, 240, L), i32),
            pltpu.VMEM((NSTEP, GP, L), i32),
            pltpu.VMEM((NSTEP, GP, L), i32),
            pltpu.VMEM((NSTEP, GP, L), i32),
            pltpu.VMEM((NSTEP, GP, L), i32),
            pltpu.VMEM((NSTEP, 24 * GH, L), f32),
            pltpu.VMEM((NSTEP, 2, L // 2, 128), i32),
            pltpu.VMEM((NSTEP, GR, L), f32),
            pltpu.VMEM((NSTEP, GR, L), f32),
            pltpu.VMEM((NT, DP, 128), i32),
            pltpu.VMEM((2 * NG, 80, 128), f32),
            pltpu.VMEM((2, 80, 128), f32),
            pltpu.VMEM((DP, F), i32),
            pltpu.VMEM((DP, F), i32),
            pltpu.VMEM((DP, F), i32),
            pltpu.VMEM((8, S), f32),
            pltpu.VMEM((5, 32, 128), f32),
            pltpu.VMEM((H, 128), f32),
            pltpu.VMEM((H, 128), f32),
            pltpu.VMEM((2 * NG, 8, L), f32),
            pltpu.VMEM((NT, 8, 128), i32),
            pltpu.VMEM((8, D), f32),
            pltpu.VMEM((8, 128), f32),
            pltpu.VMEM((8, F), f32),
            pltpu.VMEM((8, F), f32),
            pltpu.VMEM((GH, 10, 128, 128), f32),
            pltpu.VMEM((GH, 10, 128, 128), f32),
            pltpu.VMEM((GH, 4, 8, 128), f32),
            pltpu.VMEM((GH, 4, 8, 128), f32),
            pltpu.VMEM((GH, 24, 128), f32),
        ],
        compiler_params=pltpu.CompilerParams(vmem_limit_bytes=100 * 1024 * 1024),
        name="infini_mod",
    )(A_x[0].T, A_wq, A_wk, A_wv, A_wo, A_beta, B_w_r, B_w_gate, B_w_up, B_w_down.T)
    return out.T[None]
```

```python
import functools
import math

import jax
import jax.numpy as jnp
import numpy as np
from jax import lax
import jax.experimental.pallas as pl
import jax.experimental.pallas.tpu as pltpu

S, D, H, DH, NSEG, L, F = 2048, 576, 32, 18, 4, 512, 4608
DP = D // 2
GH, GR, GP = 8, 144, 72
NG = H // GH
NSTEP = NSEG * NG
NT = S // 128
FC = 512
NFC = F // FC
LOG2E = math.log2(math.e)
QSCALE = DH ** -0.5 * LOG2E
NEG = -1e9 * LOG2E
EPS_LN = float(np.asarray(1e-5, dtype=jnp.bfloat16))
ONES2 = np.int32(0x3F803F80)
IN_CHUNKS = ((0, 1), (1, 2), (2, 3), (3, 4), (4, 8), (8, 16))
OUT_CHUNKS = ((0, 4), (4, 8), (8, 12), (12, 14), (14, 15), (15, 16))
WQ_SPLIT = 384
PLAN = "q30 f p22 q31 f p20 q32 p30 f t3 p31 q20 f p00 q21 f p10 t2 q10 p21 t1 p11 q00 p33 t0 p32"
FFN_FIRST_STEP = 2

f32, bf16, i32 = jnp.float32, jnp.bfloat16, jnp.int32


def _b(x):
    return pltpu.bitcast(x, bf16)


def _w(x):
    return pltpu.bitcast(x, i32)


def _rnd(x):
    return x.astype(bf16).astype(f32)


def _phi(t):
    return jnp.where(t > 0, t + 1.0, jnp.exp(t))


def _dot(a, b):
    return jnp.dot(a, b, preferred_element_type=f32)


def _dot_nt(a, b):
    return lax.dot_general(a, b, (((1,), (1,)), ((), ())), preferred_element_type=f32)


def _iota(shape, dim):
    return lax.broadcasted_iota(i32, shape, dim)


def _between(x, lo, hi):
    return (x >= lo) & (x < hi)


def _rotate(x, quarters):
    if quarters % 4 == 0:
        return x
    tiles = [pltpu.roll(x[:, c:c + 128], 32 * (quarters % 4), 1)
             for c in range(0, x.shape[1], 128)]
    return tiles[0] if len(tiles) == 1 else jnp.concatenate(tiles, axis=1)


def _head_row(h):
    return 9 * h // 8 * 8


def _interleave(main, extra):
    done = 0
    for n, job in enumerate(main):
        job()
        while done * len(main) < (n + 1) * len(extra):
            extra[done]()
            done += 1


def _job(fn, *args, **kw):
    return functools.partial(fn, *args, **kw)


def _waits(*copies):
    def run():
        for c in copies:
            c.wait()
    return run


def _compute(x_hbm, wq_hbm, wk_hbm, wv_hbm, wo_hbm, beta_hbm, wr_hbm, wg_hbm, wu_hbm, wd_hbm,
             obuf, beta_v, wr_v, xs, xn, wraw, wq0, wq1, wqt, wkt, wvt, wot, wrt,
             qs, qsh, pqs, kt, pkt, vt, vw, kw, amem, adot, ot, mz, mmask, rden,
             wg, wu, wd, rs, sel, xsel, rsel, gu, hbuf, yacc,
             tri, gate, gate1, s_a, s_b, m_a, m_b, oacc,
             o_copy, sem_x, sem_w, sem_f):

    def x_copy(c):
        lo, hi = IN_CHUNKS[c]
        cols = pl.ds(128 * lo, 128 * (hi - lo))
        return pltpu.make_async_copy(x_hbm.bitcast(i32).at[:, cols], xs.at[:, cols], sem_x.at[c])

    def wq_copy(c):
        cols = pl.ds(0, WQ_SPLIT) if c == 0 else pl.ds(WQ_SPLIT, D - WQ_SPLIT)
        return pltpu.make_async_copy(wq_hbm.bitcast(i32).at[:, cols], (wq0, wq1)[c], sem_w.at[c])

    def w_copy(j):
        src = (wk_hbm, wv_hbm, wo_hbm)[j]
        return pltpu.make_async_copy(src.bitcast(i32), wraw.at[j], sem_w.at[2 + j])

    def small_copy(j):
        src, dst = ((beta_hbm, beta_v), (wr_hbm, wr_v))[j]
        return pltpu.make_async_copy(src, dst, sem_w.at[5 + j])

    def f_copy(j):
        src, dst = ((wg_hbm, wg), (wu_hbm, wu), (wd_hbm, wd))[j]
        return pltpu.make_async_copy(src.bitcast(i32), dst, sem_f.at[j])

    for c in (x_copy(0), wq_copy(0), x_copy(1), x_copy(2), x_copy(3), wq_copy(1), small_copy(0),
              small_copy(1), w_copy(0), w_copy(1), x_copy(4), x_copy(5), w_copy(2),
              f_copy(0), f_copy(1), f_copy(2)):
        c.start()

    def pin(i, carry):
        for ref in (s_a, s_b, m_a, m_b, kw, oacc):
            ref[i, 0, 0:8, :] = jnp.zeros((8, 128), ref.dtype)
        for ref in (qs, qsh, pqs, kt, pkt, vt, vw, amem, adot, ot, mz, tri, rden, gu):
            ref[i, 0:8, 0:128] = jnp.zeros((8, 128), ref.dtype)
        for ref in (wqt, wkt, wvt, wot, hbuf, yacc):
            ref[0:8, pl.ds(pl.multiple_of(128 * i, 128), 128)] = jnp.zeros((8, 128), ref.dtype)
        return carry

    lax.fori_loop(0, 2, pin, 0)

    key, lane = _iota((32, 128), 0), _iota((32, 128), 1)
    for a in range(4):
        tri[a] = jnp.where(key > (lane + 128 - 32 * a) % 128, NEG, 0.0)
    tri[4] = jnp.where(key > lane % 32, NEG, 0.0)
    for half in range(2):
        row, col = _iota((80, 128), 0), _iota((80, 128), 1)
        first, spare = 8 * half, 72 * (1 - half)
        keep = [_between(col, first + DH * j, first + DH * j + DH)
                & (_between(row, first + DH * j, first + DH * j + DH) | (row == spare + j))
                for j in range(4)]
        mmask[half] = jnp.where(functools.reduce(jnp.logical_or, keep), 1.0, 0.0)

    def small_inputs():
        g_row = _rnd(jax.nn.sigmoid(beta_v[...].astype(f32).reshape(1, H)))
        eye = _iota((H, H), 0) == _iota((H, H), 1)
        g_col = jnp.sum(jnp.where(eye, jnp.broadcast_to(g_row, (H, H)), 0.0), axis=1,
                        keepdims=True)
        g_all = jnp.broadcast_to(g_col, (H, 128))
        gate[...] = g_all
        gate1[...] = _rnd(1.0 - g_all)
        wr = wr_v[...].astype(f32).reshape(1, D)
        wrt[...] = _w(jnp.broadcast_to(wr, (16, D)).astype(bf16))

    def inv_std(mean, mean_r, mean_sq):
        shift = mean - mean_r
        var = jnp.maximum(mean_sq - shift * shift, 0.0)
        return 1.0 / _rnd(jnp.sqrt(_rnd(_rnd(var) + EPS_LN)))

    def layernorm(t):
        x = _b(xs[:, 128 * t:128 * t + 128]).astype(f32)
        mean = jnp.sum(x, axis=0, keepdims=True) * (1.0 / D)
        mean_r = _rnd(mean)
        xc = x - mean_r
        inv = inv_std(mean, mean_r, jnp.sum(xc * xc, axis=0, keepdims=True) * (1.0 / D))
        xn[t] = _w((_rnd(xc) * inv).astype(bf16))

    def layernorm_now(t):
        def rows(r):
            return _b(xs[r:r + 16, 128 * t:128 * t + 128]).astype(f32)

        def average(parts):
            return jnp.sum(functools.reduce(jnp.add, parts), axis=0, keepdims=True) * (1.0 / D)

        mean = average(rows(r) for r in range(0, DP, 16))
        mean_r = _rnd(mean)

        def square(r):
            xc = rows(r) - mean_r
            xn[t, r:r + 16] = _w(xc.astype(bf16))
            return xc * xc

        inv = inv_std(mean, mean_r, average(square(r) for r in range(0, DP, 16)))
        for r in range(0, DP, 16):
            xn[t, r:r + 16] = _w((_b(xn[t, r:r + 16]).astype(f32) * inv).astype(bf16))

    def score_tokens(t):
        r = _dot(_b(wrt[...]), _b(xn[t]))
        rs[:, 128 * t:128 * t + 128] = _rnd(r[0:8])

    def tiles(ref, lo, hi):
        return jnp.concatenate([ref[t] for t in range(lo, hi)], axis=1)

    def transpose_weights(j, dst):
        dst[:, 0:D] = _w(_b(wraw[j]).T)

    def proj(kind, s, g, lo=0, hi=4, w=None, fence=None):
        t, cols, n = NG * s + g, slice(128 * lo, 128 * hi), 128 * (hi - lo)
        if w is None:
            w = {"q": wqt, "k": wkt, "v": wvt}[kind][GP * g:GP * g + GP, :]
        y = _dot(_b(w), _b(tiles(xn, 4 * s + lo, 4 * s + hi)))
        if fence is not None:
            fence()
        if kind == "q":
            q = _w((y * QSCALE).astype(bf16))
            turned = {(h, r): jnp.where(_between(_iota((8, n), 0) + r, 9 * h, 9 * h + 9),
                                        _rotate(q[r:r + 8], h), 0)
                      for h in range(GH) for r in (_head_row(h), _head_row(h) + 8)}
            for (h, r), val in turned.items():
                row = 16 * h + r - _head_row(h)
                qs[t, row:row + 8, cols] = val
            quarter = _iota((8, n), 1) // 32 % 4
            for hq in (0, 4):
                for u in (1, 2, 3):
                    for r in range(8 * hq, 8 * hq + 40, 8):
                        val = 0
                        for h in range(hq, hq + 4):
                            if (h, r) in turned:
                                val = jnp.where(quarter == (u + h) % 4, turned[h, r], val)
                        row = 40 * (3 * (hq // 4) + u - 1) + r - 8 * hq
                        qsh[t, row:row + 8, cols] = val
            if s > 0:
                pqs[t, :, cols] = _w(_phi(y).astype(bf16))
        elif kind == "k":
            kt[t, :, cols] = _w(y.astype(bf16))
            if s + 1 < NSEG:
                pkt[t, :, cols] = _w(_phi(y).astype(bf16))
        else:
            if s + 1 < NSEG:
                vt[t, :, cols] = _w(y.astype(bf16))
            for h in range(GH):
                base = (DH * h) // 8 * 8
                vw[t, 24 * h:24 * h + 24, cols] = jnp.where(
                    _between(_iota((24, n), 0) + base, DH * h, DH * h + DH), y[base:base + 24], 1.0)

    def key_window(t, half):
        kw[t, half] = _w(_b(kt[t, 8 * half:8 * half + 64, :]).T)

    def mem_read(t, half):
        w = 2 * (t % NG) + half
        first, spare = 8 * half, 72 * (1 - half)
        nd = _dot(mz[w, :, 0:80].astype(bf16), _b(pqs[t, 32 * half:32 * half + 40, :]))
        gw = jnp.concatenate([gate[4 * w:4 * w + 4, :]] * 2, axis=0)
        rden[w] = jnp.tile(gw, (1, L // 128)) / (nd[spare:spare + 8] + 1e-6)
        for r in range(0, 72, 8):
            ha, hb = r // DH, (r + 7) // DH
            scale = jnp.broadcast_to(rden[w, ha:ha + 1, :], (8, L))
            if ha != hb:
                scale = jnp.where(_iota((8, L), 0) < DH * hb - r, scale,
                                  jnp.broadcast_to(rden[w, hb:hb + 1, :], (8, L)))
            amem[t, 72 * half + r:72 * half + r + 8, :] = nd[first + r:first + r + 8] * scale

    def mem_update(t, half):
        w = 2 * (t % NG) + half
        spare = 36 * (1 - half)
        v = jnp.where(_between(_iota((40, L), 0), spare, spare + 4), ONES2,
                      vt[t, 32 * half:32 * half + 40, :])
        upd = _dot_nt(_b(v), _b(pkt[t, 32 * half:32 * half + 40, :]))
        upd = jnp.where(mmask[half, :, 0:80] > 0, upd, 0.0)
        mz[w, :, 0:80] = upd if t < NG else mz[w, :, 0:80] + upd

    def post_jobs(t):
        jobs = [_job(key_window, t, half) for half in range(2)]
        if t >= NG:
            jobs += [_job(mem_read, t, half) for half in range(2)]
        if t < NSTEP - NG:
            jobs += [_job(mem_update, t, half) for half in range(2)]
        return jobs

    routed = []

    def route():
        r = rs[...]
        tok, row = _iota((8, S), 1), _iota((8, S), 0)
        m1 = jnp.max(r, axis=1, keepdims=True)
        i1 = jnp.min(jnp.where(r == m1, tok, S), axis=1, keepdims=True)
        r2 = jnp.where(tok == i1, -jnp.inf, r)
        m2 = jnp.max(r2, axis=1, keepdims=True)
        i2 = jnp.min(jnp.where((r2 == m2) & (tok != i1), tok, S), axis=1, keepdims=True)
        one = jnp.where(((row == 0) & (tok == i1)) | ((row == 1) & (tok == i2)), 1.0, 0.0)
        one = _w(jnp.concatenate([one, jnp.zeros((8, S), f32)], axis=0).astype(bf16))
        for t in range(NT):
            sel[t] = one[:, 128 * t:128 * t + 128]
        weight = _rnd(jax.nn.sigmoid(jnp.where(_iota((8, 1), 0) == 0, m1, m2)))
        rsel[...] = jnp.broadcast_to(weight, (8, 128))
        routed.extend(jnp.clip(jnp.max(i) // 128, 0, NT - 1) for i in (i1, i2))

    def gather():
        xa, xb = [_dot_nt(_b(sel[t]), _b(xn[t]))[0:8] for t in routed]
        x = jnp.where(_iota((8, D), 0) == 0, xa, xb)
        xsel[:, 0:D] = x
        xsel[:, D:D + 64] = pltpu.roll(x[:, 512:D], 2, 0)

    def ffn_up(c, j, k):
        w = (wg, wu)[j][64 * k:64 * k + 64, FC * c:FC * c + FC]
        part = _dot(xsel[:, 128 * k:128 * k + 128], _b(w).astype(f32))
        gu[j] = part if k == 0 else gu[j] + part

    def ffn_hidden(c):
        w = jnp.concatenate([m[256:DP, FC * c:FC * c + FC] for m in (wg, wu)], axis=0)
        part = _dot(xsel[:, 512:640], _b(w).astype(f32))
        g, u = _rnd(gu[0] + part), _rnd(gu[1] + pltpu.roll(part, 6, 0))
        hbuf[:, FC * c:FC * c + FC] = _rnd(_rnd(g * jax.nn.sigmoid(g)) * u)

    def ffn_down(c, n):
        w = wd[64 * n:min(64 * n + 64, DP), FC * c:FC * c + FC]
        part = _dot_nt(hbuf[:, FC * c:FC * c + FC], _b(w).astype(f32))
        cols = slice(128 * n, min(128 * n + 128, D))
        yacc[:, cols] = part if c == 0 else yacc[:, cols] + part

    def ffn_finish():
        y = jnp.where(_iota((8, D), 0) < 2, _rnd(_rnd(yacc[...]) * rsel[:, 0:1]), 0.0)
        y = jnp.concatenate([y, jnp.zeros((120, D), f32)], axis=0)
        wot[:, D:D + 16] = _w(y.T[:, 0:16].astype(bf16))

    def att_jobs(t, spare=()):
        s_w, m_w, s_r, m_r = (s_a, m_a, s_b, m_b) if t % 2 == 0 else (s_b, m_b, s_a, m_a)
        mx, sums, spare = {}, {}, list(spare)

        def keys(hq, lo, hi):
            return _b(kw[t, hq // 4, lo // 2:hi // 2, :])

        def padded(q, first):
            before, after = ([jnp.zeros((n, 128), i32)] if n else []
                             for n in (first, 64 - first - q.shape[0]))
            return _b(jnp.concatenate(before + [q] + after, axis=0))

        def vmax(sc):
            return jnp.max(sc.reshape(-1, 8, 128), axis=0)

        def scores(hq, i, j):
            full = 128 if i > 0 else 0
            part = 32 if j >= i - 1 else 0
            tile = i * (i + 1) // 2
            for h in range(hq, hq + 4):
                q = padded(qs[t, 16 * h:16 * h + 16, 128 * i:128 * i + 128], _head_row(h) - 2 * hq)
                sc = _dot(keys(hq, 128 * j, 128 * j + full + part), q)
                ms = [mx[h]] if j > 0 else []
                if full:
                    s_w[h, tile + j] = sc[0:full]
                    ms.append(vmax(sc[0:full]))
                if part:
                    d = sc[full:] + tri[h - hq]
                    s_w[h, tile + i, 0:32] = d
                    ms.append(vmax(d))
                mx[h] = functools.reduce(jnp.maximum, ms)

        def shared_scores(hq, i):
            quarter = _iota((8, 128), 1) // 32
            for u in (2, 1, 3):
                row = 40 * (3 * (hq // 4) + u - 1)
                q = padded(qsh[t, row:row + 40, 128 * i:128 * i + 128], 6 * hq)
                sc = _dot(keys(hq, 128 * i + 32, 128 * i + 32 * u + 32), q)
                d = sc[32 * u - 32:] + tri[4]
                sc = d if u == 1 else jnp.concatenate([sc[0:32 * u - 32], d], axis=0)
                s_w[hq + u, i * (i + 1) // 2 + i, 32:32 * u + 32] = sc
                mu = vmax(sc)
                for a in range(4):
                    mx[hq + a] = jnp.where(quarter == (u + a) % 4,
                                           jnp.maximum(mx[hq + a], mu), mx[hq + a])
            for h in range(hq, hq + 4):
                m_w[h, i] = jnp.broadcast_to(jnp.max(mx[h], axis=0, keepdims=True), (8, 128))

        def weights(sc, m):
            return jnp.exp2(sc.reshape(-1, 8, 128) - m[None]).reshape(sc.shape)

        def values(hq, i, j):
            tile = i * (i + 1) // 2 + j
            done = sums[hq, i] = sums.get((hq, i), 0) + 1
            shared = {}
            if j == i:
                for u in (1, 2, 3):
                    m = m_r[hq + (-u) % 4, i]
                    for p in range(1, 4):
                        m = jnp.where(_iota((8, 128), 1) // 32 == p, m_r[hq + (p - u) % 4, i], m)
                    shared[u] = weights(s_r[hq + u, tile, 32:32 * u + 32], m)
            for h in range(hq, hq + 4):
                if j < i:
                    p = weights(s_r[h, tile], m_r[h, i])
                else:
                    parts = [weights(s_r[h, tile, 0:32], m_r[h, i])]
                    for kq in (1, 2, 3):
                        x = 0.0
                        for u in range(kq, 4):
                            x = jnp.where(_iota((32, 128), 1) // 32 == (u + h) % 4,
                                          shared[u][32 * kq - 32:32 * kq], x)
                        parts.append(x)
                    p = jnp.concatenate(parts, axis=0)
                o = _dot(vw[t - 1, 24 * h:24 * h + 24, 128 * j:128 * j + 128], p)
                if done > 1:
                    o = oacc[h, i] + o
                if done <= i:
                    oacc[h, i] = o
                    continue
                base = (DH * h) // 8 * 8
                ones_row = 0 if DH * h > base else 23
                hg = GH * ((t - 1) % NG) + h
                total = jnp.broadcast_to(o[ones_row:ones_row + 1], (8, 128))
                scale = (jnp.broadcast_to(gate1[hg:hg + 1, :], (8, 128))
                         * pltpu.reciprocal(total, approx=True))
                for lo in range(base, base + 24, 8):
                    val = _rotate(o[lo - base:lo - base + 8] * scale, -h)
                    dst = adot.at[t - 1, lo:lo + 8, 128 * i:128 * i + 128]
                    if lo >= DH * h and lo + 8 <= DH * h + DH:
                        dst[...] = val
                    else:
                        pltpu.store(dst, val,
                                    mask=_between(_iota((8, 128), 0) + lo, DH * h, DH * h + DH))

        jobs = []
        for hq in (0, 4):
            for word in PLAN.split():
                at = [int(c) for c in word[1:]]
                if word[0] == "q" and t < NSTEP:
                    jobs.append(_job(scores, hq, *at))
                elif word[0] == "t" and t < NSTEP:
                    jobs.append(_job(shared_scores, hq, *at))
                elif word[0] == "p" and t > 0:
                    jobs.append(_job(values, hq, *at))
                elif word[0] == "f" and spare:
                    jobs.append(spare.pop(0))
        return jobs

    def pack_heads(t):
        o = adot[t] if t < NG else adot[t] + amem[t]
        o = _w(o.astype(bf16))
        for c in range(4):
            ot[4 * (t // NG) + c, GP * (t % NG):GP * (t % NG) + GP] = o[:, 128 * c:128 * c + 128]

    def out_proj(c, r):
        lo, hi = OUT_CHUNKS[c]
        rows = slice(r, r + GP)
        rhs = jnp.concatenate([tiles(ot, lo, hi), tiles(sel, lo, hi)], axis=0)
        y = _dot(_b(wot[rows, 0:D + 16]), _b(rhs))
        if c > 0 and r == 0:
            o_copy(c - 1).start()
        xnc = jnp.concatenate([xn[t, rows] for t in range(lo, hi)], axis=1)
        y = y + (_b(xs[rows, 128 * lo:128 * hi]).astype(f32) + _b(xnc).astype(f32))
        obuf[rows, 128 * lo:128 * hi] = _w(y.astype(bf16))

    def out_jobs(c):
        return [_job(out_proj, c, r) for r in range(0, DP, GP)]

    x_copy(0).wait()
    layernorm_now(0)
    wq_copy(0).wait()
    w = _w(_b(wq0[...]).T)
    wqt[0:WQ_SPLIT // 2, :] = w
    proj("q", 0, 0, 0, 1, w=w[0:GP])
    proj("q", 0, 1, 0, 1, w=w[GP:2 * GP], fence=_waits(x_copy(1), x_copy(2)))
    for t in (1, 2):
        layernorm_now(t)
        proj("q", 0, 0, t, t + 1)
        proj("q", 0, 1, t, t + 1, fence=(
            _waits(x_copy(3), wq_copy(1), small_copy(0), small_copy(1)) if t == 2 else None))
    wqt[WQ_SPLIT // 2:, :] = _w(_b(wq1[...]).T)
    layernorm_now(3)
    small_inputs()
    proj("q", 0, 2, 0, 3)
    for g in range(3):
        proj("q", 0, g, 3, 4, fence=_waits(w_copy(0)) if g == 2 else None)
    transpose_weights(0, wkt)
    proj("q", 0, 3)
    for g in range(NG):
        proj("k", 0, g, fence=_waits(w_copy(1) if g == 2 else x_copy(4)) if g >= 2 else None)
        if g == 2:
            transpose_weights(1, wvt)
        score_tokens(g)
    for g in range(NG):
        layernorm(4 + g)
        proj("v", 0, g)
        score_tokens(4 + g)

    for t in range(NG, NSTEP):
        s, g = divmod(t, NG)
        extra = sum((post_jobs(u) for u in (range(NG) if t == NG else [t - 1])), [])
        if s + 1 < NSEG:
            extra.insert(1, _job(layernorm, t + NG))
            extra.append(_job(score_tokens, t + NG))
        elif g < 3:
            extra.insert(1, (_job(transpose_weights, 2, wot), route, gather)[g])
        fence = _waits(x_copy(5), w_copy(2)) if t == NG else None
        _interleave([_job(proj, "q", s, g, fence=fence), _job(proj, "k", s, g),
                     _job(proj, "v", s, g)], extra)

    ffn_work = []
    for c in range(NFC + 1):
        up = [_job(ffn_up, c, j, k) for j in range(2) for k in range(4)] + [_job(ffn_hidden, c)]
        for n in range(5):
            if c < NFC:
                ffn_work += up[2 * n:2 * n + 2]
            if c > 0:
                ffn_work.append(_job(ffn_down, c - 1, n))
    ffn_work.append(ffn_finish)
    slots = 2 * PLAN.count("f")
    assert len(ffn_work) <= slots * (NSTEP - FFN_FIRST_STEP)

    _interleave(att_jobs(0), post_jobs(NSTEP - 1))
    for t in range(1, NSTEP):
        if t == FFN_FIRST_STEP:
            _waits(f_copy(0), f_copy(1), f_copy(2))()
        if t >= 2:
            pack_heads(t - 2)
        first = slots * (t - FFN_FIRST_STEP)
        for job in att_jobs(t, ffn_work[first:first + slots] if first >= 0 else ()):
            job()

    _interleave(out_jobs(0), [_job(pack_heads, NSTEP - 2)] + att_jobs(NSTEP))
    pack_heads(NSTEP - 1)
    for c in range(1, len(OUT_CHUNKS)):
        for job in out_jobs(c):
            job()
    o_copy(len(OUT_CHUNKS) - 1).start()


def _kernel(*refs):
    inputs, (out_hbm, sem_o, obuf), scratch = refs[:10], refs[10:13], refs[13:]

    def o_copy(c):
        lo, hi = OUT_CHUNKS[c]
        cols = pl.ds(128 * lo, 128 * (hi - lo))
        return pltpu.make_async_copy(obuf.at[:, cols], out_hbm.bitcast(i32).at[:, cols], sem_o)

    pl.run_scoped(functools.partial(_compute, *inputs, obuf, *scratch, o_copy),
                  pltpu.SemaphoreType.DMA((len(IN_CHUNKS),)), pltpu.SemaphoreType.DMA((7,)),
                  pltpu.SemaphoreType.DMA((3,)))
    for c in range(len(OUT_CHUNKS)):
        o_copy(c).wait()


@jax.jit
def pallas_parallel_sum__memory_aug_infini_attn__moe_arch_mod__prompt_kernel(
    A_x, A_wq, A_wk, A_wv, A_wo, A_beta, B_x, B_w_r, B_w_gate, B_w_up, B_w_down,
):
    del B_x
    hbm = pl.BlockSpec(memory_space=pl.ANY)
    out = pl.pallas_call(
        _kernel,
        out_shape=jax.ShapeDtypeStruct((D, S), bf16),
        in_specs=[hbm] * 10,
        out_specs=hbm,
        scratch_shapes=[
            pltpu.SemaphoreType.DMA(()),
            pltpu.VMEM((DP, S), i32),
            pltpu.VMEM((H,), bf16),
            pltpu.VMEM((D,), bf16),
            pltpu.VMEM((DP, S), i32),
            pltpu.VMEM((NT, DP, 128), i32),
            pltpu.VMEM((3, DP, D), i32),
            pltpu.VMEM((DP, WQ_SPLIT), i32),
            pltpu.VMEM((DP, D - WQ_SPLIT), i32),
            pltpu.VMEM((DP, D), i32),
            pltpu.VMEM((DP, D), i32),
            pltpu.VMEM((DP, D), i32),
            pltpu.VMEM((DP, 640), i32),
            pltpu.VMEM((8, D), i32),
            pltpu.VMEM((NSTEP, 16 * GH, L), i32),
            pltpu.VMEM((NSTEP, 240, L), i32),
            pltpu.VMEM((NSTEP, GP, L), i32),
            pltpu.VMEM((NSTEP, GP, L), i32),
            pltpu.VMEM((NSTEP, GP, L), i32),
            pltpu.VMEM((NSTEP, GP, L), i32),
            pltpu.VMEM((NSTEP, 24 * GH, L), f32),
            pltpu.VMEM((NSTEP, 2, L // 2, 128), i32),
            pltpu.VMEM((NSTEP, GR, L), f32),
            pltpu.VMEM((NSTEP, GR, L), f32),
            pltpu.VMEM((NT, DP, 128), i32),
            pltpu.VMEM((2 * NG, 80, 128), f32),
            pltpu.VMEM((2, 80, 128), f32),
            pltpu.VMEM((2 * NG, 8, L), f32),
            pltpu.VMEM((DP, F), i32),
            pltpu.VMEM((DP, F), i32),
            pltpu.VMEM((DP, F), i32),
            pltpu.VMEM((8, S), f32),
            pltpu.VMEM((NT, 8, 128), i32),
            pltpu.VMEM((8, 640), f32),
            pltpu.VMEM((8, 128), f32),
            pltpu.VMEM((2, 8, FC), f32),
            pltpu.VMEM((8, F), f32),
            pltpu.VMEM((8, D), f32),
            pltpu.VMEM((5, 32, 128), f32),
            pltpu.VMEM((H, 128), f32),
            pltpu.VMEM((H, 128), f32),
            pltpu.VMEM((GH, 10, 128, 128), f32),
            pltpu.VMEM((GH, 10, 128, 128), f32),
            pltpu.VMEM((GH, 4, 8, 128), f32),
            pltpu.VMEM((GH, 4, 8, 128), f32),
            pltpu.VMEM((GH, 4, 24, 128), f32),
        ],
        compiler_params=pltpu.CompilerParams(vmem_limit_bytes=100 * 1024 * 1024),
        name="infini_mod",
    )(A_x[0].T, A_wq, A_wk, A_wv, A_wo, A_beta, B_w_r, B_w_gate, B_w_up, B_w_down.T)
    return out.T[None]
```

```python
import functools
import math

import jax
import jax.numpy as jnp
import numpy as np
from jax import lax
import jax.experimental.pallas as pl
import jax.experimental.pallas.tpu as pltpu

S, D, H, DH, NSEG, L, F = 2048, 576, 32, 18, 4, 512, 4608
DP = D // 2
GH, GR, GP = 8, 144, 72
NG = H // GH
NSTEP = NSEG * NG
NT = S // 128
FC = 512
NFC = F // FC
LOG2E = math.log2(math.e)
QSCALE = DH ** -0.5 * LOG2E
NEG = -1e9 * LOG2E
EPS_LN = float(np.asarray(1e-5, dtype=jnp.bfloat16))
ONES2 = np.int32(0x3F803F80)
IN_CHUNKS = ((0, 1), (1, 2), (2, 3), (3, 4), (4, 8), (8, 16))
OUT_CHUNKS = ((0, 8), (8, 12), (12, 14), (14, 15), (15, 16))
WQ_SPLIT = 384
PLAN = "q30 f p22 q31 f p20 q32 p30 f t3 p31 q20 f p00 q21 f p10 t2 q10 p21 t1 p11 q00 p33 t0 p32"
FFN_FIRST_STEP = 2

f32, bf16, i32 = jnp.float32, jnp.bfloat16, jnp.int32


def _b(x):
    return pltpu.bitcast(x, bf16)


def _w(x):
    return pltpu.bitcast(x, i32)


def _rnd(x):
    return x.astype(bf16).astype(f32)


def _phi(t):
    return jnp.where(t > 0, t + 1.0, jnp.exp(t))


def _dot(a, b):
    return jnp.dot(a, b, preferred_element_type=f32)


def _dot_nt(a, b):
    return lax.dot_general(a, b, (((1,), (1,)), ((), ())), preferred_element_type=f32)


def _iota(shape, dim):
    return lax.broadcasted_iota(i32, shape, dim)


def _between(x, lo, hi):
    return (x >= lo) & (x < hi)


def _rotate(x, quarters):
    if quarters % 4 == 0:
        return x
    tiles = [pltpu.roll(x[:, c:c + 128], 32 * (quarters % 4), 1)
             for c in range(0, x.shape[1], 128)]
    return tiles[0] if len(tiles) == 1 else jnp.concatenate(tiles, axis=1)


def _head_row(h):
    return 9 * h // 8 * 8


def _interleave(main, extra):
    done = 0
    for n, job in enumerate(main):
        job()
        while done * len(main) < (n + 1) * len(extra):
            extra[done]()
            done += 1


def _job(fn, *args, **kw):
    return functools.partial(fn, *args, **kw)


def _waits(*copies):
    def run():
        for c in copies:
            c.wait()
    return run


def _compute(x_hbm, wq_hbm, wk_hbm, wv_hbm, wo_hbm, beta_hbm, wr_hbm, wg_hbm, wu_hbm, wd_hbm,
             obuf, beta_v, wr_v, xs, xn, wraw, wq0, wq1, wqt, wkt, wvt, wot, wrt,
             qs, qsh, pqs, kt, pkt, vt, vw, kw, nd, adot, ot, mz, mmask,
             wg, wu, wd, rs, sel, xsel, rsel, gu, hbuf, yacc,
             tri, gate, gate1, s_a, s_b, m_a, m_b, oacc,
             o_copy, sem_x, sem_w, sem_f):

    def x_copy(c):
        lo, hi = IN_CHUNKS[c]
        cols = pl.ds(128 * lo, 128 * (hi - lo))
        return pltpu.make_async_copy(x_hbm.bitcast(i32).at[:, cols], xs.at[:, cols], sem_x.at[c])

    def wq_copy(c):
        cols = pl.ds(0, WQ_SPLIT) if c == 0 else pl.ds(WQ_SPLIT, D - WQ_SPLIT)
        return pltpu.make_async_copy(wq_hbm.bitcast(i32).at[:, cols], (wq0, wq1)[c], sem_w.at[c])

    def w_copy(j):
        src = (wk_hbm, wv_hbm, wo_hbm)[j]
        return pltpu.make_async_copy(src.bitcast(i32), wraw.at[j], sem_w.at[2 + j])

    def small_copy(j):
        src, dst = ((beta_hbm, beta_v), (wr_hbm, wr_v))[j]
        return pltpu.make_async_copy(src, dst, sem_w.at[5 + j])

    def f_copy(j):
        src, dst = ((wg_hbm, wg), (wu_hbm, wu), (wd_hbm, wd))[j]
        return pltpu.make_async_copy(src.bitcast(i32), dst, sem_f.at[j])

    for c in (x_copy(0), wq_copy(0), x_copy(1), x_copy(2), x_copy(3), wq_copy(1), small_copy(0),
              small_copy(1), w_copy(0), w_copy(1), x_copy(4), x_copy(5), w_copy(2),
              f_copy(0), f_copy(1), f_copy(2)):
        c.start()

    def pin(i, carry):
        for ref in (s_a, s_b, m_a, m_b, kw, oacc, nd):
            ref[i, 0, 0:8, 0:128] = jnp.zeros((8, 128), ref.dtype)
        for ref in (qs, qsh, pqs, kt, pkt, vt, vw, adot, ot, mz, tri, gu):
            ref[i, 0:8, 0:128] = jnp.zeros((8, 128), ref.dtype)
        for ref in (wqt, wkt, wvt, wot, hbuf, yacc):
            ref[0:8, pl.ds(pl.multiple_of(128 * i, 128), 128)] = jnp.zeros((8, 128), ref.dtype)
        return carry

    lax.fori_loop(0, 2, pin, 0)

    key, lane = _iota((32, 128), 0), _iota((32, 128), 1)
    for a in range(4):
        tri[a] = jnp.where(key > (lane + 128 - 32 * a) % 128, NEG, 0.0)
    tri[4] = jnp.where(key > lane % 32, NEG, 0.0)
    for half in range(2):
        row, col = _iota((80, 128), 0), _iota((80, 128), 1)
        first, spare = 8 * half, 72 * (1 - half)
        keep = [_between(col, first + DH * j, first + DH * j + DH)
                & (_between(row, first + DH * j, first + DH * j + DH) | (row == spare + j))
                for j in range(4)]
        mmask[half] = jnp.where(functools.reduce(jnp.logical_or, keep), 1.0, 0.0)

    @functools.cache
    def quarter(rows, cols, p):
        return (_iota((rows, cols), 1) >> 5) & 3 == p

    @functools.cache
    def row_range(rows, cols, lo, hi):
        return _between(_iota((rows, cols), 0), lo, hi)

    def small_inputs():
        g_row = _rnd(jax.nn.sigmoid(beta_v[...].astype(f32).reshape(1, H)))
        eye = _iota((H, H), 0) == _iota((H, H), 1)
        g_col = jnp.sum(jnp.where(eye, jnp.broadcast_to(g_row, (H, H)), 0.0), axis=1,
                        keepdims=True)
        g_all = jnp.broadcast_to(g_col, (H, 128))
        gate[...] = g_all
        gate1[...] = _rnd(1.0 - g_all)
        wr = wr_v[...].astype(f32).reshape(1, D)
        wrt[...] = _w(jnp.broadcast_to(wr, (16, D)).astype(bf16))

    def inv_std(mean, mean_r, mean_sq):
        shift = mean - mean_r
        var = jnp.maximum(mean_sq - shift * shift, 0.0)
        return 1.0 / _rnd(jnp.sqrt(_rnd(_rnd(var) + EPS_LN)))

    def layernorm(t):
        x = _b(xs[:, 128 * t:128 * t + 128]).astype(f32)
        mean = jnp.sum(x, axis=0, keepdims=True) * (1.0 / D)
        mean_r = _rnd(mean)
        xc = x - mean_r
        inv = inv_std(mean, mean_r, jnp.sum(xc * xc, axis=0, keepdims=True) * (1.0 / D))
        xn[t] = _w((_rnd(xc) * inv).astype(bf16))

    def layernorm_now(t):
        def rows(r):
            return _b(xs[r:r + 16, 128 * t:128 * t + 128]).astype(f32)

        def average(parts):
            return jnp.sum(functools.reduce(jnp.add, parts), axis=0, keepdims=True) * (1.0 / D)

        mean = average(rows(r) for r in range(0, DP, 16))
        mean_r = _rnd(mean)

        def square(r):
            xc = rows(r) - mean_r
            xn[t, r:r + 16] = _w(xc.astype(bf16))
            return xc * xc

        inv = inv_std(mean, mean_r, average(square(r) for r in range(0, DP, 16)))
        for r in range(0, DP, 16):
            xn[t, r:r + 16] = _w((_b(xn[t, r:r + 16]).astype(f32) * inv).astype(bf16))

    def score_tokens(t):
        r = _dot(_b(wrt[...]), _b(xn[t]))
        rs[:, 128 * t:128 * t + 128] = _rnd(r[0:8])

    def tiles(ref, lo, hi):
        return jnp.concatenate([ref[t] for t in range(lo, hi)], axis=1)

    def transpose_weights(j, dst):
        dst[:, 0:D] = _w(_b(wraw[j]).T)

    def proj(kind, s, g, lo=0, hi=4, w=None, fence=None):
        t, cols, n = NG * s + g, slice(128 * lo, 128 * hi), 128 * (hi - lo)
        if w is None:
            w = {"q": wqt, "k": wkt, "v": wvt}[kind][GP * g:GP * g + GP, :]
        y = _dot(_b(w), _b(tiles(xn, 4 * s + lo, 4 * s + hi)))
        if fence is not None:
            fence()
        if kind == "q":
            q = _w((y * QSCALE).astype(bf16))
            turned = {(h, r): jnp.where(row_range(8, n, 9 * h - r, 9 * h + 9 - r),
                                        _rotate(q[r:r + 8], h), 0)
                      for h in range(GH) for r in (_head_row(h), _head_row(h) + 8)}
            for (h, r), val in turned.items():
                row = 16 * h + r - _head_row(h)
                qs[t, row:row + 8, cols] = val
            for hq in (0, 4):
                for u in (1, 2, 3):
                    for r in range(8 * hq, 8 * hq + 40, 8):
                        val = 0
                        for h in range(hq, hq + 4):
                            if (h, r) in turned:
                                val = jnp.where(quarter(8, n, (u + h) % 4), turned[h, r], val)
                        row = 40 * (3 * (hq // 4) + u - 1) + r - 8 * hq
                        qsh[t, row:row + 8, cols] = val
            if s > 0:
                pqs[t, :, cols] = _w(_phi(y).astype(bf16))
        elif kind == "k":
            kt[t, :, cols] = _w(y.astype(bf16))
            if s + 1 < NSEG:
                pkt[t, :, cols] = _w(_phi(y).astype(bf16))
        else:
            if s + 1 < NSEG:
                vt[t, :, cols] = _w(y.astype(bf16))
            for h in range(GH):
                base = (DH * h) // 8 * 8
                vw[t, 24 * h:24 * h + 24, cols] = jnp.where(
                    row_range(24, n, DH * h - base, DH * h + DH - base), y[base:base + 24], 1.0)

    def key_window(t, half):
        kw[t, half] = _w(_b(kt[t, 8 * half:8 * half + 64, :]).T)

    def mem_read(t, half):
        m = mz[2 * (t % NG) + half, :, 0:80].astype(bf16)
        nd[t, half] = _dot(m, _b(pqs[t, 32 * half:32 * half + 40, :]))

    def mem_output(t, half):
        w = 2 * (t % NG) + half
        first, spare = 8 * half, 72 * (1 - half)
        gw = jnp.concatenate([gate[4 * w:4 * w + 4, :]] * 2, axis=0)
        rden = jnp.tile(gw, (1, L // 128)) / (nd[t, half, spare:spare + 8, :] + 1e-6)
        rden = [jnp.broadcast_to(rden[h:h + 1], (8, L)) for h in range(4)]
        rows = []
        for r in range(0, 72, 8):
            ha, hb = r // DH, (r + 7) // DH
            scale = rden[ha]
            if ha != hb:
                scale = jnp.where(row_range(8, L, 0, DH * hb - r), scale, rden[hb])
            rows.append(nd[t, half, first + r:first + r + 8, :] * scale)
        return rows

    def mem_update(t, half):
        w = 2 * (t % NG) + half
        spare = 36 * (1 - half)
        v = jnp.where(row_range(40, L, spare, spare + 4), ONES2, vt[t, 32 * half:32 * half + 40, :])
        upd = _dot_nt(_b(v), _b(pkt[t, 32 * half:32 * half + 40, :]))
        upd = jnp.where(mmask[half, :, 0:80] > 0, upd, 0.0)
        mz[w, :, 0:80] = upd if t < NG else mz[w, :, 0:80] + upd

    def post_jobs(t):
        jobs = [_job(key_window, t, half) for half in range(2)]
        if t >= NG:
            jobs += [_job(mem_read, t, half) for half in range(2)]
        if t < NSTEP - NG:
            jobs += [_job(mem_update, t, half) for half in range(2)]
        return jobs

    routed = []

    def route():
        r = rs[...]
        tok, row = _iota((8, S), 1), _iota((8, S), 0)
        m1 = jnp.max(r, axis=1, keepdims=True)
        i1 = jnp.min(jnp.where(r == m1, tok, S), axis=1, keepdims=True)
        r2 = jnp.where(tok == i1, -jnp.inf, r)
        m2 = jnp.max(r2, axis=1, keepdims=True)
        i2 = jnp.min(jnp.where((r2 == m2) & (tok != i1), tok, S), axis=1, keepdims=True)
        one = jnp.where(((row == 0) & (tok == i1)) | ((row == 1) & (tok == i2)), 1.0, 0.0)
        one = _w(jnp.concatenate([one, jnp.zeros((8, S), f32)], axis=0).astype(bf16))
        for t in range(NT):
            sel[t] = one[:, 128 * t:128 * t + 128]
        weight = _rnd(jax.nn.sigmoid(jnp.where(_iota((8, 1), 0) == 0, m1, m2)))
        rsel[...] = jnp.broadcast_to(weight, (8, 128))
        routed.extend(jnp.clip(jnp.max(i) // 128, 0, NT - 1) for i in (i1, i2))

    def gather():
        xa, xb = [_dot_nt(_b(sel[t]), _b(xn[t]))[0:8] for t in routed]
        x = jnp.where(_iota((8, D), 0) == 0, xa, xb)
        xsel[:, 0:D] = x
        xsel[:, D:D + 64] = pltpu.roll(x[:, 512:D], 2, 0)

    def ffn_up(c, j, k):
        w = (wg, wu)[j][64 * k:64 * k + 64, FC * c:FC * c + FC]
        part = _dot(xsel[:, 128 * k:128 * k + 128], _b(w).astype(f32))
        gu[j] = part if k == 0 else gu[j] + part

    def ffn_hidden(c):
        w = jnp.concatenate([m[256:DP, FC * c:FC * c + FC] for m in (wg, wu)], axis=0)
        part = _dot(xsel[:, 512:640], _b(w).astype(f32))
        g, u = _rnd(gu[0] + part), _rnd(gu[1] + pltpu.roll(part, 6, 0))
        hbuf[:, FC * c:FC * c + FC] = _rnd(_rnd(g * jax.nn.sigmoid(g)) * u)

    def ffn_down(c, n):
        w = wd[64 * n:min(64 * n + 64, DP), FC * c:FC * c + FC]
        part = _dot_nt(hbuf[:, FC * c:FC * c + FC], _b(w).astype(f32))
        cols = slice(128 * n, min(128 * n + 128, D))
        yacc[:, cols] = part if c == 0 else yacc[:, cols] + part

    def ffn_finish():
        y = jnp.where(_iota((8, D), 0) < 2, _rnd(_rnd(yacc[...]) * rsel[:, 0:1]), 0.0)
        y = jnp.concatenate([y, jnp.zeros((120, D), f32)], axis=0)
        wot[:, D:D + 16] = _w(y.T[:, 0:16].astype(bf16))

    def att_jobs(t, spare=()):
        s_w, m_w, s_r, m_r = (s_a, m_a, s_b, m_b) if t % 2 == 0 else (s_b, m_b, s_a, m_a)
        mx, sums, spare = {}, {}, list(spare)

        def keys(hq, lo, hi):
            return _b(kw[t, hq // 4, lo // 2:hi // 2, :])

        def padded(q, first):
            before, after = ([jnp.zeros((n, 128), i32)] if n else []
                             for n in (first, 64 - first - q.shape[0]))
            return _b(jnp.concatenate(before + [q] + after, axis=0))

        def vmax(sc):
            return jnp.max(sc.reshape(-1, 8, 128), axis=0)

        def scores(hq, i, j):
            full = 128 if i > 0 else 0
            part = 32 if j >= i - 1 else 0
            tile = i * (i + 1) // 2
            for h in range(hq, hq + 4):
                q = padded(qs[t, 16 * h:16 * h + 16, 128 * i:128 * i + 128], _head_row(h) - 2 * hq)
                sc = _dot(keys(hq, 128 * j, 128 * j + full + part), q)
                ms = [mx[h]] if j > 0 else []
                if full:
                    s_w[h, tile + j] = sc[0:full]
                    ms.append(vmax(sc[0:full]))
                if part:
                    d = sc[full:] + tri[h - hq]
                    s_w[h, tile + i, 0:32] = d
                    ms.append(vmax(d))
                mx[h] = functools.reduce(jnp.maximum, ms)

        def shared_scores(hq, i):
            for u in (2, 1, 3):
                row = 40 * (3 * (hq // 4) + u - 1)
                q = padded(qsh[t, row:row + 40, 128 * i:128 * i + 128], 6 * hq)
                sc = _dot(keys(hq, 128 * i + 32, 128 * i + 32 * u + 32), q)
                d = sc[32 * u - 32:] + tri[4]
                sc = d if u == 1 else jnp.concatenate([sc[0:32 * u - 32], d], axis=0)
                s_w[hq + u, i * (i + 1) // 2 + i, 32:32 * u + 32] = sc
                mu = vmax(sc)
                for a in range(4):
                    mx[hq + a] = jnp.where(quarter(8, 128, (u + a) % 4),
                                           jnp.maximum(mx[hq + a], mu), mx[hq + a])
            for h in range(hq, hq + 4):
                m_w[h, i] = jnp.broadcast_to(jnp.max(mx[h], axis=0, keepdims=True), (8, 128))

        def weights(sc, m):
            return jnp.exp2(sc.reshape(-1, 8, 128) - m[None]).reshape(sc.shape)

        def values(hq, i, j):
            tile = i * (i + 1) // 2 + j
            done = sums[hq, i] = sums.get((hq, i), 0) + 1
            shared = {}
            if j == i:
                for u in (1, 2, 3):
                    m = m_r[hq + (-u) % 4, i]
                    for p in range(1, 4):
                        m = jnp.where(quarter(8, 128, p), m_r[hq + (p - u) % 4, i], m)
                    shared[u] = weights(s_r[hq + u, tile, 32:32 * u + 32], m)
            for h in range(hq, hq + 4):
                if j < i:
                    p = weights(s_r[h, tile], m_r[h, i])
                else:
                    parts = [weights(s_r[h, tile, 0:32], m_r[h, i])]
                    for kq in (1, 2, 3):
                        x = 0.0
                        for u in range(kq, 4):
                            x = jnp.where(quarter(32, 128, (u + h) % 4),
                                          shared[u][32 * kq - 32:32 * kq], x)
                        parts.append(x)
                    p = jnp.concatenate(parts, axis=0)
                o = _dot(vw[t - 1, 24 * h:24 * h + 24, 128 * j:128 * j + 128], p)
                if done > 1:
                    o = oacc[h, i] + o
                if done <= i:
                    oacc[h, i] = o
                    continue
                base = (DH * h) // 8 * 8
                ones_row = 0 if DH * h > base else 23
                hg = GH * ((t - 1) % NG) + h
                total = jnp.broadcast_to(o[ones_row:ones_row + 1], (8, 128))
                scale = (jnp.broadcast_to(gate1[hg:hg + 1, :], (8, 128))
                         * pltpu.reciprocal(total, approx=True))
                for lo in range(base, base + 24, 8):
                    val = _rotate(o[lo - base:lo - base + 8] * scale, -h)
                    dst = adot.at[t - 1, lo:lo + 8, 128 * i:128 * i + 128]
                    if lo >= DH * h and lo + 8 <= DH * h + DH:
                        dst[...] = val
                    else:
                        pltpu.store(dst, val,
                                    mask=row_range(8, 128, DH * h - lo, DH * h + DH - lo))

        jobs = []
        for hq in (0, 4):
            for word in PLAN.split():
                at = [int(c) for c in word[1:]]
                if word[0] == "q" and t < NSTEP:
                    jobs.append(_job(scores, hq, *at))
                elif word[0] == "t" and t < NSTEP:
                    jobs.append(_job(shared_scores, hq, *at))
                elif word[0] == "p" and t > 0:
                    jobs.append(_job(values, hq, *at))
                elif word[0] == "f" and spare:
                    jobs.append(spare.pop(0))
        return jobs

    def pack_heads(t):
        o = adot[t]
        if t >= NG:
            o = o + jnp.concatenate(mem_output(t, 0) + mem_output(t, 1), axis=0)
        o = _w(o.astype(bf16))
        for c in range(4):
            ot[4 * (t // NG) + c, GP * (t % NG):GP * (t % NG) + GP] = o[:, 128 * c:128 * c + 128]

    def out_proj(c, r):
        lo, hi = OUT_CHUNKS[c]
        rows = slice(r, r + GP)
        rhs = jnp.concatenate([tiles(ot, lo, hi), tiles(sel, lo, hi)], axis=0)
        y = _dot(_b(wot[rows, 0:D + 16]), _b(rhs))
        if c > 0 and r == 0:
            o_copy(c - 1).start()
        xnc = jnp.concatenate([xn[t, rows] for t in range(lo, hi)], axis=1)
        y = y + (_b(xs[rows, 128 * lo:128 * hi]).astype(f32) + _b(xnc).astype(f32))
        obuf[rows, 128 * lo:128 * hi] = _w(y.astype(bf16))

    def out_jobs(c):
        return [_job(out_proj, c, r) for r in range(0, DP, GP)]

    x_copy(0).wait()
    layernorm_now(0)
    wq_copy(0).wait()
    w = _w(_b(wq0[...]).T)
    wqt[0:WQ_SPLIT // 2, :] = w
    proj("q", 0, 0, 0, 1, w=w[0:GP])
    proj("q", 0, 1, 0, 1, w=w[GP:2 * GP], fence=_waits(x_copy(1), x_copy(2)))
    for t in (1, 2):
        layernorm_now(t)
        proj("q", 0, 0, t, t + 1)
        proj("q", 0, 1, t, t + 1, fence=(
            _waits(x_copy(3), wq_copy(1), small_copy(0), small_copy(1)) if t == 2 else None))
    wqt[WQ_SPLIT // 2:, :] = _w(_b(wq1[...]).T)
    layernorm_now(3)
    small_inputs()
    proj("q", 0, 2, 0, 3)
    for g in range(3):
        proj("q", 0, g, 3, 4, fence=_waits(w_copy(0)) if g == 2 else None)
    transpose_weights(0, wkt)
    proj("q", 0, 3)
    for g in range(NG):
        proj("k", 0, g, fence=_waits(w_copy(1) if g == 2 else x_copy(4)) if g >= 2 else None)
        if g == 2:
            transpose_weights(1, wvt)
        score_tokens(g)
    for g in range(NG):
        layernorm(4 + g)
        proj("v", 0, g)
        score_tokens(4 + g)

    for t in range(NG, NSTEP):
        s, g = divmod(t, NG)
        extra = sum((post_jobs(u) for u in (range(NG) if t == NG else [t - 1])), [])
        if s + 1 < NSEG:
            extra.insert(1, _job(layernorm, t + NG))
            extra.append(_job(score_tokens, t + NG))
        elif g < 2:
            extra.insert(1, (_job(transpose_weights, 2, wot), route)[g])
        fence = _waits(x_copy(5), w_copy(2)) if t == NG else None
        _interleave([_job(proj, "q", s, g, fence=fence), _job(proj, "k", s, g),
                     _job(proj, "v", s, g)], extra)

    ffn_work = []
    for c in range(NFC + 1):
        up = [_job(ffn_up, c, j, k) for j in range(2) for k in range(4)] + [_job(ffn_hidden, c)]
        for n in range(5):
            if c < NFC:
                ffn_work += up[2 * n:2 * n + 2]
            if c > 0:
                ffn_work.append(_job(ffn_down, c - 1, n))
    ffn_work.append(ffn_finish)
    slots = 2 * PLAN.count("f")
    assert len(ffn_work) <= slots * (NSTEP - FFN_FIRST_STEP)

    _interleave(att_jobs(0), post_jobs(NSTEP - 1) + [gather])
    for t in range(1, NSTEP):
        if t == FFN_FIRST_STEP:
            _waits(f_copy(0), f_copy(1), f_copy(2))()
        if t >= 2:
            pack_heads(t - 2)
        first = slots * (t - FFN_FIRST_STEP)
        for job in att_jobs(t, ffn_work[first:first + slots] if first >= 0 else ()):
            job()

    _interleave(out_jobs(0), [_job(pack_heads, NSTEP - 2)] + att_jobs(NSTEP))
    pack_heads(NSTEP - 1)
    for c in range(1, len(OUT_CHUNKS)):
        for job in out_jobs(c):
            job()
    o_copy(len(OUT_CHUNKS) - 1).start()


def _kernel(*refs):
    inputs, (out_hbm, sem_o, obuf), scratch = refs[:10], refs[10:13], refs[13:]

    def o_copy(c):
        lo, hi = OUT_CHUNKS[c]
        cols = pl.ds(128 * lo, 128 * (hi - lo))
        return pltpu.make_async_copy(obuf.at[:, cols], out_hbm.bitcast(i32).at[:, cols], sem_o)

    pl.run_scoped(functools.partial(_compute, *inputs, obuf, *scratch, o_copy),
                  pltpu.SemaphoreType.DMA((len(IN_CHUNKS),)), pltpu.SemaphoreType.DMA((7,)),
                  pltpu.SemaphoreType.DMA((3,)))
    for c in range(len(OUT_CHUNKS)):
        o_copy(c).wait()


@jax.jit
def pallas_parallel_sum__memory_aug_infini_attn__moe_arch_mod__prompt_kernel(
    A_x, A_wq, A_wk, A_wv, A_wo, A_beta, B_x, B_w_r, B_w_gate, B_w_up, B_w_down,
):
    del B_x
    hbm = pl.BlockSpec(memory_space=pl.ANY)
    out = pl.pallas_call(
        _kernel,
        out_shape=jax.ShapeDtypeStruct((D, S), bf16),
        in_specs=[hbm] * 10,
        out_specs=hbm,
        scratch_shapes=[
            pltpu.SemaphoreType.DMA(()),
            pltpu.VMEM((DP, S), i32),
            pltpu.VMEM((H,), bf16),
            pltpu.VMEM((D,), bf16),
            pltpu.VMEM((DP, S), i32),
            pltpu.VMEM((NT, DP, 128), i32),
            pltpu.VMEM((3, DP, D), i32),
            pltpu.VMEM((DP, WQ_SPLIT), i32),
            pltpu.VMEM((DP, D - WQ_SPLIT), i32),
            pltpu.VMEM((DP, D), i32),
            pltpu.VMEM((DP, D), i32),
            pltpu.VMEM((DP, D), i32),
            pltpu.VMEM((DP, 640), i32),
            pltpu.VMEM((8, D), i32),
            pltpu.VMEM((NSTEP, 16 * GH, L), i32),
            pltpu.VMEM((NSTEP, 240, L), i32),
            pltpu.VMEM((NSTEP, GP, L), i32),
            pltpu.VMEM((NSTEP, GP, L), i32),
            pltpu.VMEM((NSTEP, GP, L), i32),
            pltpu.VMEM((NSTEP, GP, L), i32),
            pltpu.VMEM((NSTEP, 24 * GH, L), f32),
            pltpu.VMEM((NSTEP, 2, L // 2, 128), i32),
            pltpu.VMEM((NSTEP, 2, 80, L), f32),
            pltpu.VMEM((NSTEP, GR, L), f32),
            pltpu.VMEM((NT, DP, 128), i32),
            pltpu.VMEM((2 * NG, 80, 128), f32),
            pltpu.VMEM((2, 80, 128), f32),
            pltpu.VMEM((DP, F), i32),
            pltpu.VMEM((DP, F), i32),
            pltpu.VMEM((DP, F), i32),
            pltpu.VMEM((8, S), f32),
            pltpu.VMEM((NT, 8, 128), i32),
            pltpu.VMEM((8, 640), f32),
            pltpu.VMEM((8, 128), f32),
            pltpu.VMEM((2, 8, FC), f32),
            pltpu.VMEM((8, F), f32),
            pltpu.VMEM((8, D), f32),
            pltpu.VMEM((5, 32, 128), f32),
            pltpu.VMEM((H, 128), f32),
            pltpu.VMEM((H, 128), f32),
            pltpu.VMEM((GH, 10, 128, 128), f32),
            pltpu.VMEM((GH, 10, 128, 128), f32),
            pltpu.VMEM((GH, 4, 8, 128), f32),
            pltpu.VMEM((GH, 4, 8, 128), f32),
            pltpu.VMEM((GH, 4, 24, 128), f32),
        ],
        compiler_params=pltpu.CompilerParams(vmem_limit_bytes=100 * 1024 * 1024),
        name="infini_mod",
    )(A_x[0].T, A_wq, A_wk, A_wv, A_wo, A_beta, B_w_r, B_w_gate, B_w_up, B_w_down.T)
    return out.T[None]
```

```python
import functools
import math

import jax
import jax.numpy as jnp
import numpy as np
from jax import lax
import jax.experimental.pallas as pl
import jax.experimental.pallas.tpu as pltpu

S, D, H, DH, NSEG, L, F = 2048, 576, 32, 18, 4, 512, 4608
DP = D // 2
GH, GR, GP = 8, 144, 72
NG = H // GH
NSTEP = NSEG * NG
NT = S // 128
FC = 512
NFC = F // FC
LOG2E = math.log2(math.e)
QSCALE = DH ** -0.5 * LOG2E
NEG = -1e9 * LOG2E
EPS_LN = float(np.asarray(1e-5, dtype=jnp.bfloat16))
ONES2 = np.int32(0x3F803F80)
IN_CHUNKS = ((0, 1), (1, 2), (2, 3), (3, 4), (4, 8), (8, 16))
OUT_CHUNKS = ((0, 8), (8, 12), (12, 14), (14, 15), (15, 16))
WQ_SPLIT = 384
PLAN = "q30 f p22 q31 f p20 q32 p30 f t3 p31 q20 f p00 q21 f p10 t2 q10 p21 t1 p11 q00 p33 t0 p32"
FFN_FIRST_STEP = 2

f32, bf16, i32 = jnp.float32, jnp.bfloat16, jnp.int32


def _b(x):
    return pltpu.bitcast(x, bf16)


def _w(x):
    return pltpu.bitcast(x, i32)


def _rnd(x):
    return x.astype(bf16).astype(f32)


def _phi(t):
    return jnp.where(t > 0, t + 1.0, jnp.exp(t))


def _dot(a, b):
    return jnp.dot(a, b, preferred_element_type=f32)


def _dot_nt(a, b):
    return lax.dot_general(a, b, (((1,), (1,)), ((), ())), preferred_element_type=f32)


def _iota(shape, dim):
    return lax.broadcasted_iota(i32, shape, dim)


def _between(x, lo, hi):
    return (x >= lo) & (x < hi)


def _rotate(x, quarters):
    if quarters % 4 == 0:
        return x
    tiles = [pltpu.roll(x[:, c:c + 128], 32 * (quarters % 4), 1)
             for c in range(0, x.shape[1], 128)]
    return tiles[0] if len(tiles) == 1 else jnp.concatenate(tiles, axis=1)


def _head_row(h):
    return 9 * h // 8 * 8


def _interleave(main, extra):
    done = 0
    for n, job in enumerate(main):
        job()
        while done * len(main) < (n + 1) * len(extra):
            extra[done]()
            done += 1


def _job(fn, *args, **kw):
    return functools.partial(fn, *args, **kw)


def _waits(*copies):
    def run():
        for c in copies:
            c.wait()
    return run


def _compute(x_hbm, wq_hbm, wk_hbm, wv_hbm, wo_hbm, beta_hbm, wr_hbm, wg_hbm, wu_hbm, wd_hbm,
             obuf, beta_v, wr_v, xs, xn, wraw, wq0, wq1, wqt, wkt, wvt, wot, wrt,
             qs, qsh, pqs, kt, pkt, vt, vw, kw, nd, adot, ot, mz, mmask,
             wg, wu, wd, rs, sel, xsel, rsel, gu, hbuf, yacc,
             tri, gate, gate1, s_a, s_b, m_a, m_b, oacc,
             o_copy, sem_x, sem_w, sem_f):

    def x_copy(c):
        lo, hi = IN_CHUNKS[c]
        cols = pl.ds(128 * lo, 128 * (hi - lo))
        return pltpu.make_async_copy(x_hbm.bitcast(i32).at[:, cols], xs.at[:, cols], sem_x.at[c])

    def wq_copy(c):
        cols = pl.ds(0, WQ_SPLIT) if c == 0 else pl.ds(WQ_SPLIT, D - WQ_SPLIT)
        return pltpu.make_async_copy(wq_hbm.bitcast(i32).at[:, cols], (wq0, wq1)[c], sem_w.at[c])

    def w_copy(j):
        src = (wk_hbm, wv_hbm, wo_hbm)[j]
        return pltpu.make_async_copy(src.bitcast(i32), wraw.at[j], sem_w.at[2 + j])

    def small_copy(j):
        src, dst = ((beta_hbm, beta_v), (wr_hbm, wr_v))[j]
        return pltpu.make_async_copy(src, dst, sem_w.at[5 + j])

    def f_copy(j):
        src, dst = ((wg_hbm, wg), (wu_hbm, wu), (wd_hbm, wd))[j]
        return pltpu.make_async_copy(src.bitcast(i32), dst, sem_f.at[j])

    for c in (x_copy(0), wq_copy(0), x_copy(1), x_copy(2), x_copy(3), wq_copy(1), small_copy(0),
              small_copy(1), w_copy(0), w_copy(1), x_copy(4), x_copy(5), w_copy(2),
              f_copy(0), f_copy(1), f_copy(2)):
        c.start()

    def pin(i, carry):
        for ref in (s_a, s_b, m_a, m_b, kw, oacc, nd):
            ref[i, 0, 0:8, 0:128] = jnp.zeros((8, 128), ref.dtype)
        for ref in (qs, qsh, pqs, kt, pkt, vt, vw, adot, ot, mz, tri, gu):
            ref[i, 0:8, 0:128] = jnp.zeros((8, 128), ref.dtype)
        for ref in (wqt, wkt, wvt, wot, hbuf, yacc):
            ref[0:8, pl.ds(pl.multiple_of(128 * i, 128), 128)] = jnp.zeros((8, 128), ref.dtype)
        return carry

    lax.fori_loop(0, 2, pin, 0)

    key, lane = _iota((32, 128), 0), _iota((32, 128), 1)
    for a in range(4):
        tri[a] = jnp.where(key > (lane + 128 - 32 * a) % 128, NEG, 0.0)
    tri[4] = jnp.where(key > lane % 32, NEG, 0.0)
    for half in range(2):
        row, col = _iota((80, 128), 0), _iota((80, 128), 1)
        first, spare = 8 * half, 72 * (1 - half)
        keep = [_between(col, first + DH * j, first + DH * j + DH)
                & (_between(row, first + DH * j, first + DH * j + DH) | (row == spare + j))
                for j in range(4)]
        mmask[half] = jnp.where(functools.reduce(jnp.logical_or, keep), 1.0, 0.0)

    @functools.cache
    def quarter(rows, cols, p):
        return (_iota((rows, cols), 1) >> 5) & 3 == p

    @functools.cache
    def row_range(rows, cols, lo, hi):
        return _between(_iota((rows, cols), 0), lo, hi)

    def small_inputs():
        g_row = _rnd(jax.nn.sigmoid(beta_v[...].astype(f32).reshape(1, H)))
        eye = _iota((H, H), 0) == _iota((H, H), 1)
        g_col = jnp.sum(jnp.where(eye, jnp.broadcast_to(g_row, (H, H)), 0.0), axis=1,
                        keepdims=True)
        g_all = jnp.broadcast_to(g_col, (H, 128))
        gate[...] = g_all
        gate1[...] = _rnd(1.0 - g_all)
        wr = wr_v[...].astype(f32).reshape(1, D)
        wrt[...] = _w(jnp.broadcast_to(wr, (16, D)).astype(bf16))

    def inv_std(mean, mean_r, mean_sq):
        shift = mean - mean_r
        var = jnp.maximum(mean_sq - shift * shift, 0.0)
        return 1.0 / _rnd(jnp.sqrt(_rnd(_rnd(var) + EPS_LN)))

    def layernorm(t):
        x = _b(xs[:, 128 * t:128 * t + 128]).astype(f32)
        mean = jnp.sum(x, axis=0, keepdims=True) * (1.0 / D)
        mean_r = _rnd(mean)
        xc = x - mean_r
        inv = inv_std(mean, mean_r, jnp.sum(xc * xc, axis=0, keepdims=True) * (1.0 / D))
        xn[t] = _w((_rnd(xc) * inv).astype(bf16))

    def layernorm_now(t):
        def rows(r):
            return _b(xs[r:r + 16, 128 * t:128 * t + 128]).astype(f32)

        def average(parts):
            return jnp.sum(functools.reduce(jnp.add, parts), axis=0, keepdims=True) * (1.0 / D)

        mean = average(rows(r) for r in range(0, DP, 16))
        mean_r = _rnd(mean)

        def square(r):
            xc = rows(r) - mean_r
            xn[t, r:r + 16] = _w(xc.astype(bf16))
            return xc * xc

        inv = inv_std(mean, mean_r, average(square(r) for r in range(0, DP, 16)))
        for r in range(0, DP, 16):
            xn[t, r:r + 16] = _w((_b(xn[t, r:r + 16]).astype(f32) * inv).astype(bf16))

    def score_tokens(t):
        r = _dot(_b(wrt[...]), _b(xn[t]))
        rs[:, 128 * t:128 * t + 128] = _rnd(r[0:8])

    def tiles(ref, lo, hi):
        return jnp.concatenate([ref[t] for t in range(lo, hi)], axis=1)

    def transpose_weights(j, dst):
        dst[:, 0:D] = _w(_b(wraw[j]).T)

    def proj(kind, s, g, lo=0, hi=4, w=None, fence=None):
        t, cols, n = NG * s + g, slice(128 * lo, 128 * hi), 128 * (hi - lo)
        if w is None:
            w = {"q": wqt, "k": wkt, "v": wvt}[kind][GP * g:GP * g + GP, :]
        y = _dot(_b(w), _b(tiles(xn, 4 * s + lo, 4 * s + hi)))
        if fence is not None:
            fence()
        if kind == "q":
            q = _w((y * QSCALE).astype(bf16))
            turned = {(h, r): jnp.where(row_range(8, n, 9 * h - r, 9 * h + 9 - r),
                                        _rotate(q[r:r + 8], h), 0)
                      for h in range(GH) for r in (_head_row(h), _head_row(h) + 8)}
            for (h, r), val in turned.items():
                row = 16 * h + r - _head_row(h)
                qs[t, row:row + 8, cols] = val
            for hq in (0, 4):
                for u in (1, 2, 3):
                    for r in range(8 * hq, 8 * hq + 40, 8):
                        val = 0
                        for h in range(hq, hq + 4):
                            if (h, r) in turned:
                                val = jnp.where(quarter(8, n, (u + h) % 4), turned[h, r], val)
                        row = 40 * (3 * (hq // 4) + u - 1) + r - 8 * hq
                        qsh[t, row:row + 8, cols] = val
            if s > 0:
                pqs[t, :, cols] = _w(_phi(y).astype(bf16))
        elif kind == "k":
            kt[t, :, cols] = _w(y.astype(bf16))
            if s + 1 < NSEG:
                pkt[t, :, cols] = _w(_phi(y).astype(bf16))
        else:
            if s + 1 < NSEG:
                vt[t, :, cols] = _w(y.astype(bf16))
            for h in range(GH):
                base = (DH * h) // 8 * 8
                vw[t, 24 * h:24 * h + 24, cols] = jnp.where(
                    row_range(24, n, DH * h - base, DH * h + DH - base), y[base:base + 24], 1.0)

    def key_window(t, half):
        kw[t, half] = _w(_b(kt[t, 8 * half:8 * half + 64, :]).T)

    def mem_read(t, half):
        m = mz[2 * (t % NG) + half, :, 0:80].astype(bf16)
        nd[t, half] = _dot(m, _b(pqs[t, 32 * half:32 * half + 40, :]))

    def mem_output(t, half):
        w = 2 * (t % NG) + half
        first, spare = 8 * half, 72 * (1 - half)
        gw = jnp.concatenate([gate[4 * w:4 * w + 4, :]] * 2, axis=0)
        rden = jnp.tile(gw, (1, L // 128)) / (nd[t, half, spare:spare + 8, :] + 1e-6)
        rden = [jnp.broadcast_to(rden[h:h + 1], (8, L)) for h in range(4)]
        rows = []
        for r in range(0, 72, 8):
            ha, hb = r // DH, (r + 7) // DH
            scale = rden[ha]
            if ha != hb:
                scale = jnp.where(row_range(8, L, 0, DH * hb - r), scale, rden[hb])
            rows.append(nd[t, half, first + r:first + r + 8, :] * scale)
        return rows

    def mem_update(t, half):
        w = 2 * (t % NG) + half
        spare = 36 * (1 - half)
        v = jnp.where(row_range(40, L, spare, spare + 4), ONES2, vt[t, 32 * half:32 * half + 40, :])
        upd = _dot_nt(_b(v), _b(pkt[t, 32 * half:32 * half + 40, :]))
        upd = jnp.where(mmask[half, :, 0:80] > 0, upd, 0.0)
        mz[w, :, 0:80] = upd if t < NG else mz[w, :, 0:80] + upd

    def post_jobs(t):
        jobs = [_job(key_window, t, half) for half in range(2)]
        if t >= NG:
            jobs += [_job(mem_read, t, half) for half in range(2)]
        if t < NSTEP - NG:
            jobs += [_job(mem_update, t, half) for half in range(2)]
        return jobs

    routed = []

    def route():
        r = rs[...]
        tok, row = _iota((8, S), 1), _iota((8, S), 0)
        m1 = jnp.max(r, axis=1, keepdims=True)
        i1 = jnp.min(jnp.where(r == m1, tok, S), axis=1, keepdims=True)
        r2 = jnp.where(tok == i1, -jnp.inf, r)
        m2 = jnp.max(r2, axis=1, keepdims=True)
        i2 = jnp.min(jnp.where((r2 == m2) & (tok != i1), tok, S), axis=1, keepdims=True)
        one = jnp.where(((row == 0) & (tok == i1)) | ((row == 1) & (tok == i2)), 1.0, 0.0)
        one = _w(jnp.concatenate([one, jnp.zeros((8, S), f32)], axis=0).astype(bf16))
        for t in range(NT):
            sel[t] = one[:, 128 * t:128 * t + 128]
        weight = _rnd(jax.nn.sigmoid(jnp.where(_iota((8, 1), 0) == 0, m1, m2)))
        rsel[...] = jnp.broadcast_to(weight, (8, 128))
        routed.extend(jnp.clip(jnp.max(i) // 128, 0, NT - 1) for i in (i1, i2))

    def gather():
        xa, xb = [_dot_nt(_b(sel[t]), _b(xn[t]))[0:8] for t in routed]
        x = jnp.where(_iota((8, D), 0) == 0, xa, xb)
        xsel[:, 0:D] = x
        xsel[:, D:D + 64] = pltpu.roll(x[:, 512:D], 2, 0)

    def ffn_up(c, j, k):
        w = (wg, wu)[j][64 * k:64 * k + 64, FC * c:FC * c + FC]
        part = _dot(xsel[:, 128 * k:128 * k + 128], _b(w).astype(f32))
        gu[j] = part if k == 0 else gu[j] + part

    def ffn_hidden(c):
        w = jnp.concatenate([m[256:DP, FC * c:FC * c + FC] for m in (wg, wu)], axis=0)
        part = _dot(xsel[:, 512:640], _b(w).astype(f32))
        g, u = _rnd(gu[0] + part), _rnd(gu[1] + pltpu.roll(part, 6, 0))
        hbuf[:, FC * c:FC * c + FC] = _rnd(_rnd(g * jax.nn.sigmoid(g)) * u)

    def ffn_down(c, n):
        w = wd[64 * n:min(64 * n + 64, DP), FC * c:FC * c + FC]
        part = _dot_nt(hbuf[:, FC * c:FC * c + FC], _b(w).astype(f32))
        cols = slice(128 * n, min(128 * n + 128, D))
        yacc[:, cols] = part if c == 0 else yacc[:, cols] + part

    def ffn_finish():
        y = jnp.where(_iota((8, D), 0) < 2, _rnd(_rnd(yacc[...]) * rsel[:, 0:1]), 0.0)
        y = jnp.concatenate([y, jnp.zeros((120, D), f32)], axis=0)
        wot[:, D:D + 16] = _w(y.T[:, 0:16].astype(bf16))

    def att_jobs(t, spare=()):
        s_w, m_w, s_r, m_r = (s_a, m_a, s_b, m_b) if t % 2 == 0 else (s_b, m_b, s_a, m_a)
        mx, sums, spare = {}, {}, list(spare)

        def keys(hq, lo, hi):
            return _b(kw[t, hq // 4, lo // 2:hi // 2, :])

        def padded(q, first):
            before, after = ([jnp.zeros((n, 128), i32)] if n else []
                             for n in (first, 64 - first - q.shape[0]))
            return _b(jnp.concatenate(before + [q] + after, axis=0))

        def vmax(sc):
            return jnp.max(sc.reshape(-1, 8, 128), axis=0)

        def scores(hq, i, j):
            full = 128 if i > 0 else 0
            part = 32 if j >= i - 1 else 0
            tile = i * (i + 1) // 2
            for h in range(hq, hq + 4):
                q = padded(qs[t, 16 * h:16 * h + 16, 128 * i:128 * i + 128], _head_row(h) - 2 * hq)
                sc = _dot(keys(hq, 128 * j, 128 * j + full + part), q)
                ms = [mx[h]] if j > 0 else []
                if full:
                    s_w[h, tile + j] = sc[0:full]
                    ms.append(vmax(sc[0:full]))
                if part:
                    d = sc[full:] + tri[h - hq]
                    s_w[h, tile + i, 0:32] = d
                    ms.append(vmax(d))
                mx[h] = functools.reduce(jnp.maximum, ms)

        def shared_scores(hq, i):
            for u in (2, 1, 3):
                row = 40 * (3 * (hq // 4) + u - 1)
                q = padded(qsh[t, row:row + 40, 128 * i:128 * i + 128], 6 * hq)
                sc = _dot(keys(hq, 128 * i + 32, 128 * i + 32 * u + 32), q)
                d = sc[32 * u - 32:] + tri[4]
                sc = d if u == 1 else jnp.concatenate([sc[0:32 * u - 32], d], axis=0)
                s_w[hq + u, i * (i + 1) // 2 + i, 32:32 * u + 32] = sc
                mu = vmax(sc)
                for a in range(4):
                    mx[hq + a] = jnp.where(quarter(8, 128, (u + a) % 4),
                                           jnp.maximum(mx[hq + a], mu), mx[hq + a])
            for h in range(hq, hq + 4):
                m_w[h, i] = jnp.broadcast_to(jnp.max(mx[h], axis=0, keepdims=True), (8, 128))

        def weights(sc, m):
            return jnp.exp2(sc.reshape(-1, 8, 128) - m[None]).reshape(sc.shape)

        def values(hq, i, j):
            tile = i * (i + 1) // 2 + j
            done = sums[hq, i] = sums.get((hq, i), 0) + 1
            shared = {}
            if j == i:
                for u in (1, 2, 3):
                    m = m_r[hq + (-u) % 4, i]
                    for p in range(1, 4):
                        m = jnp.where(quarter(8, 128, p), m_r[hq + (p - u) % 4, i], m)
                    shared[u] = weights(s_r[hq + u, tile, 32:32 * u + 32], m)
            for h in range(hq, hq + 4):
                if j < i:
                    p = weights(s_r[h, tile], m_r[h, i])
                else:
                    parts = [weights(s_r[h, tile, 0:32], m_r[h, i])]
                    for kq in (1, 2, 3):
                        x = 0.0
                        for u in range(kq, 4):
                            x = jnp.where(quarter(32, 128, (u + h) % 4),
                                          shared[u][32 * kq - 32:32 * kq], x)
                        parts.append(x)
                    p = jnp.concatenate(parts, axis=0)
                o = _dot(vw[t - 1, 24 * h:24 * h + 24, 128 * j:128 * j + 128], p)
                if done > 1:
                    o = oacc[h, i] + o
                if done <= i:
                    oacc[h, i] = o
                    continue
                base = (DH * h) // 8 * 8
                ones_row = 0 if DH * h > base else 23
                hg = GH * ((t - 1) % NG) + h
                scale = (jnp.broadcast_to(gate1[hg:hg + 1, :], (8, 128))
                         / jnp.broadcast_to(o[ones_row:ones_row + 1], (8, 128)))
                for lo in range(base, base + 24, 8):
                    val = _rotate(o[lo - base:lo - base + 8] * scale, -h)
                    dst = adot.at[t - 1, lo:lo + 8, 128 * i:128 * i + 128]
                    if lo >= DH * h and lo + 8 <= DH * h + DH:
                        dst[...] = val
                    else:
                        pltpu.store(dst, val,
                                    mask=row_range(8, 128, DH * h - lo, DH * h + DH - lo))

        jobs = []
        for hq in (0, 4):
            for word in PLAN.split():
                at = [int(c) for c in word[1:]]
                if word[0] == "q" and t < NSTEP:
                    jobs.append(_job(scores, hq, *at))
                elif word[0] == "t" and t < NSTEP:
                    jobs.append(_job(shared_scores, hq, *at))
                elif word[0] == "p" and t > 0:
                    jobs.append(_job(values, hq, *at))
                elif word[0] == "f" and spare:
                    jobs.append(spare.pop(0))
        return jobs

    def pack_heads(t):
        o = adot[t]
        if t >= NG:
            o = o + jnp.concatenate(mem_output(t, 0) + mem_output(t, 1), axis=0)
        o = _w(o.astype(bf16))
        for c in range(4):
            ot[4 * (t // NG) + c, GP * (t % NG):GP * (t % NG) + GP] = o[:, 128 * c:128 * c + 128]

    def out_proj(c, r):
        lo, hi = OUT_CHUNKS[c]
        rows = slice(r, r + GP)
        rhs = jnp.concatenate([tiles(ot, lo, hi), tiles(sel, lo, hi)], axis=0)
        y = _dot(_b(wot[rows, 0:D + 16]), _b(rhs))
        if c > 0 and r == 0:
            o_copy(c - 1).start()
        xnc = jnp.concatenate([xn[t, rows] for t in range(lo, hi)], axis=1)
        y = y + (_b(xs[rows, 128 * lo:128 * hi]).astype(f32) + _b(xnc).astype(f32))
        obuf[rows, 128 * lo:128 * hi] = _w(y.astype(bf16))

    def out_jobs(c):
        return [_job(out_proj, c, r) for r in range(0, DP, GP)]

    x_copy(0).wait()
    layernorm_now(0)
    wq_copy(0).wait()
    w = _w(_b(wq0[...]).T)
    wqt[0:WQ_SPLIT // 2, :] = w
    proj("q", 0, 0, 0, 1, w=w[0:GP], fence=_waits(x_copy(1)))
    proj("q", 0, 1, 0, 1)
    layernorm_now(1)
    proj("q", 0, 0, 1, 2, fence=_waits(x_copy(2), x_copy(3)))
    proj("q", 0, 1, 1, 2)
    layernorm_now(2)
    proj("q", 0, 0, 2, 3)
    proj("q", 0, 1, 2, 3, fence=_waits(wq_copy(1), small_copy(0), small_copy(1)))
    wqt[WQ_SPLIT // 2:, :] = _w(_b(wq1[...]).T)
    layernorm_now(3)
    small_inputs()
    proj("q", 0, 2, 0, 3)
    for g in range(3):
        proj("q", 0, g, 3, 4, fence=_waits(w_copy(0)) if g == 2 else None)
    transpose_weights(0, wkt)
    proj("q", 0, 3)
    for g in range(NG):
        proj("k", 0, g, fence=_waits(w_copy(1), x_copy(4)) if g == 3 else None)
        if g == 3:
            transpose_weights(1, wvt)
        score_tokens(g)
    for g in range(NG):
        layernorm(4 + g)
        proj("v", 0, g)
        score_tokens(4 + g)

    for t in range(NG, NSTEP):
        s, g = divmod(t, NG)
        extra = sum((post_jobs(u) for u in (range(NG) if t == NG else [t - 1])), [])
        if s + 1 < NSEG:
            extra.insert(1, _job(layernorm, t + NG))
            extra.append(_job(score_tokens, t + NG))
        elif g < 2:
            extra.insert(1, (_job(transpose_weights, 2, wot), route)[g])
        fence = _waits(x_copy(5), w_copy(2)) if t == NG else None
        _interleave([_job(proj, "q", s, g, fence=fence), _job(proj, "k", s, g),
                     _job(proj, "v", s, g)], extra)

    ffn_work = []
    for c in range(NFC + 1):
        up = [_job(ffn_up, c, j, k) for j in range(2) for k in range(4)] + [_job(ffn_hidden, c)]
        for n in range(5):
            if c < NFC:
                ffn_work += up[2 * n:2 * n + 2]
            if c > 0:
                ffn_work.append(_job(ffn_down, c - 1, n))
    ffn_work.append(ffn_finish)
    slots = 2 * PLAN.count("f")
    assert len(ffn_work) <= slots * (NSTEP - FFN_FIRST_STEP)

    _interleave(att_jobs(0), post_jobs(NSTEP - 1) + [gather])
    for t in range(1, NSTEP):
        if t == FFN_FIRST_STEP:
            _waits(f_copy(0), f_copy(1), f_copy(2))()
        if t >= 2:
            pack_heads(t - 2)
        first = slots * (t - FFN_FIRST_STEP)
        for job in att_jobs(t, ffn_work[first:first + slots] if first >= 0 else ()):
            job()

    _interleave(out_jobs(0), [_job(pack_heads, NSTEP - 2)] + att_jobs(NSTEP))
    pack_heads(NSTEP - 1)
    for c in range(1, len(OUT_CHUNKS)):
        for job in out_jobs(c):
            job()
    o_copy(len(OUT_CHUNKS) - 1).start()


def _kernel(*refs):
    inputs, (out_hbm, sem_o, obuf), scratch = refs[:10], refs[10:13], refs[13:]

    def o_copy(c):
        lo, hi = OUT_CHUNKS[c]
        cols = pl.ds(128 * lo, 128 * (hi - lo))
        return pltpu.make_async_copy(obuf.at[:, cols], out_hbm.bitcast(i32).at[:, cols], sem_o)

    pl.run_scoped(functools.partial(_compute, *inputs, obuf, *scratch, o_copy),
                  pltpu.SemaphoreType.DMA((len(IN_CHUNKS),)), pltpu.SemaphoreType.DMA((7,)),
                  pltpu.SemaphoreType.DMA((3,)))
    for c in range(len(OUT_CHUNKS)):
        o_copy(c).wait()


@jax.jit
def pallas_parallel_sum__memory_aug_infini_attn__moe_arch_mod__prompt_kernel(
    A_x, A_wq, A_wk, A_wv, A_wo, A_beta, B_x, B_w_r, B_w_gate, B_w_up, B_w_down,
):
    del B_x
    hbm = pl.BlockSpec(memory_space=pl.ANY)
    out = pl.pallas_call(
        _kernel,
        out_shape=jax.ShapeDtypeStruct((D, S), bf16),
        in_specs=[hbm] * 10,
        out_specs=hbm,
        scratch_shapes=[
            pltpu.SemaphoreType.DMA(()),
            pltpu.VMEM((DP, S), i32),
            pltpu.VMEM((H,), bf16),
            pltpu.VMEM((D,), bf16),
            pltpu.VMEM((DP, S), i32),
            pltpu.VMEM((NT, DP, 128), i32),
            pltpu.VMEM((3, DP, D), i32),
            pltpu.VMEM((DP, WQ_SPLIT), i32),
            pltpu.VMEM((DP, D - WQ_SPLIT), i32),
            pltpu.VMEM((DP, D), i32),
            pltpu.VMEM((DP, D), i32),
            pltpu.VMEM((DP, D), i32),
            pltpu.VMEM((DP, 640), i32),
            pltpu.VMEM((8, D), i32),
            pltpu.VMEM((NSTEP, 16 * GH, L), i32),
            pltpu.VMEM((NSTEP, 240, L), i32),
            pltpu.VMEM((NSTEP, GP, L), i32),
            pltpu.VMEM((NSTEP, GP, L), i32),
            pltpu.VMEM((NSTEP, GP, L), i32),
            pltpu.VMEM((NSTEP, GP, L), i32),
            pltpu.VMEM((NSTEP, 24 * GH, L), f32),
            pltpu.VMEM((NSTEP, 2, L // 2, 128), i32),
            pltpu.VMEM((NSTEP, 2, 80, L), f32),
            pltpu.VMEM((NSTEP, GR, L), f32),
            pltpu.VMEM((NT, DP, 128), i32),
            pltpu.VMEM((2 * NG, 80, 128), f32),
            pltpu.VMEM((2, 80, 128), f32),
            pltpu.VMEM((DP, F), i32),
            pltpu.VMEM((DP, F), i32),
            pltpu.VMEM((DP, F), i32),
            pltpu.VMEM((8, S), f32),
            pltpu.VMEM((NT, 8, 128), i32),
            pltpu.VMEM((8, 640), f32),
            pltpu.VMEM((8, 128), f32),
            pltpu.VMEM((2, 8, FC), f32),
            pltpu.VMEM((8, F), f32),
            pltpu.VMEM((8, D), f32),
            pltpu.VMEM((5, 32, 128), f32),
            pltpu.VMEM((H, 128), f32),
            pltpu.VMEM((H, 128), f32),
            pltpu.VMEM((GH, 10, 128, 128), f32),
            pltpu.VMEM((GH, 10, 128, 128), f32),
            pltpu.VMEM((GH, 4, 8, 128), f32),
            pltpu.VMEM((GH, 4, 8, 128), f32),
            pltpu.VMEM((GH, 4, 24, 128), f32),
        ],
        compiler_params=pltpu.CompilerParams(vmem_limit_bytes=100 * 1024 * 1024),
        name="infini_mod",
    )(A_x[0].T, A_wq, A_wk, A_wv, A_wo, A_beta, B_w_r, B_w_gate, B_w_up, B_w_down.T)
    return out.T[None]
```
